```python
import jax
import jax.numpy as jnp

def _softmax(x, axis=-1):
    return jax.nn.softmax(x, axis=axis)

def _gelu(x):
    return jax.nn.gelu(x, approximate=True)

def _silu(x):
    return jax.nn.silu(x)

def _sigmoid(x):
    return jax.nn.sigmoid(x)

def _layernorm(x, axis=-1, eps=1e-05):
    m = jnp.mean(x, axis=axis, keepdims=True)
    v = jnp.var(x, axis=axis, keepdims=True)
    return (x - m) / jnp.sqrt(v + eps)

def _scatter_add(tgt, idx, src, axis=0):
    return tgt.at[idx].add(src)

def _segment_sum(src, seg, n):
    return jax.ops.segment_sum(src, seg, n)

class _Rng:

    def __init__(self, key):
        self._k = key

    def _next(self):
        self._k, sub = jax.random.split(self._k)
        return sub

    def normal(self, shape):
        return jax.random.normal(self._next(), shape, dtype=jnp.bfloat16)

    def randint(self, lo, hi, shape):
        return jax.random.randint(self._next(), shape, lo, hi, dtype=jnp.int32)

    def uniform(self, shape, lo=0.0, hi=1.0):
        return jax.random.uniform(self._next(), shape, jnp.bfloat16, lo, hi)

    def permutation(self, n):
        return jax.random.permutation(self._next(), n)
kernel_name = 'interleave_layers__memory_aug_recurrent_mem_tr__spectral_gfnet__prompt'

def setup_inputs():
    _rng = _Rng(jax.random.key(int.from_bytes(__import__("os").urandom(4), "little")))
    _w = lambda a: (lambda t: t.astype(jnp.bfloat16) if jnp.issubdtype(t.dtype, jnp.floating) else t)(jnp.asarray(a))

    def _A_setup():
        B, S, Dm = (1, 2048, 640)
        H, Dh = (32, 128)
        M, seg = (8, 32)
        seg = min(seg, S)
        S = S // seg * seg
        return {'x': _w((lambda *s: _rng.normal(s) * 0.05)(B, S, Dm)), 'mem0': _w((lambda *s: _rng.normal(s) * 0.05)(B, M, Dm)), 'Wq': _w((lambda *s: _rng.normal(s) * 0.05)(Dm, H, Dh) * Dm ** (-0.5)), 'Wk': _w((lambda *s: _rng.normal(s) * 0.05)(Dm, H, Dh) * Dm ** (-0.5)), 'Wv': _w((lambda *s: _rng.normal(s) * 0.05)(Dm, H, Dh) * Dm ** (-0.5)), 'Wo': _w((lambda *s: _rng.normal(s) * 0.05)(H, Dh, Dm) * (H * Dh) ** (-0.5)), 'seg_len': seg}
    _A_in = _A_setup()

    def _B_setup():
        B, S, D = (1, 2048, 640)
        Df = D // 2 + 1
        return {'x': _w((lambda *s: _rng.normal(s) * 0.05)(B, S, D)), 'w_r': _w((lambda *s: _rng.normal(s) * 0.05)(S, Df) * 0.02), 'w_i': _w((lambda *s: _rng.normal(s) * 0.05)(S, Df) * 0.02)}
    _B_in = _B_setup()
    return {'A_x': _A_in['x'], 'A_mem0': _A_in['mem0'], 'A_Wq': _A_in['Wq'], 'A_Wk': _A_in['Wk'], 'A_Wv': _A_in['Wv'], 'A_Wo': _A_in['Wo'], 'A_seg_len': _A_in['seg_len'], 'B_x': _B_in['x'], 'B_w_r': _B_in['w_r'], 'B_w_i': _B_in['w_i']}

def reference(A_x, A_mem0, A_Wq, A_Wk, A_Wv, A_Wo, A_seg_len, B_x, B_w_r, B_w_i):

    def _A_ref(x, mem0, Wq, Wk, Wv, Wo, seg_len):
        B, S, Dm = x.shape
        H, Dh = (Wq.shape[1], Wq.shape[2])
        M = mem0.shape[1]
        scale = Dh ** (-0.5)
        n_seg = S // seg_len
        L = M + seg_len
        idx = jnp.arange(L)
        mask = (idx[:, None] < M) | (idx[:, None] >= idx[None, :])
        mem = mem0
        outs = []
        for s in range(n_seg):
            xs = x[:, s * seg_len:(s + 1) * seg_len, :].copy()
            h = jnp.concatenate([mem, xs], axis=1)
            q = jnp.einsum('btd,dhe->bhte', h, Wq)
            k = jnp.einsum('btd,dhe->bhte', h, Wk)
            v = jnp.einsum('btd,dhe->bhte', h, Wv)
            scores = jnp.einsum('bhqe,bhke->bhqk', q, k) * scale
            scores = jnp.where(mask[None, None], scores, -1000000000.0)
            p = _softmax(scores, axis=-1)
            o = jnp.einsum('bhqk,bhke->bhqe', p, v)
            o = jnp.einsum('bhte,hed->btd', o, Wo)
            mem = o[:, :M, :].copy()
            outs.append(o[:, M:, :])
        return jnp.concatenate(outs, axis=1)

    def _B_ref(x, w_r, w_i):
        B, S, D = x.shape
        X = (lambda x, axes=(-2, -1): jnp.fft.rfft2(x.astype(jnp.float32), axes=axes))(x, axes=(-2, -1))
        W = w_r + 1j * w_i
        X = X * W
        y = (lambda x, s, axes=(-2, -1): jnp.fft.irfft2(x, s=s, axes=axes).astype(jnp.bfloat16))(X, (S, D), axes=(-2, -1))
        return y
    x = A_x
    x = x + _A_ref(_layernorm(x, axis=-1), A_mem0, A_Wq, A_Wk, A_Wv, A_Wo, A_seg_len)
    x = x + _B_ref(_layernorm(x, axis=-1), B_w_r, B_w_i)
    x = x + _A_ref(_layernorm(x, axis=-1), A_mem0, A_Wq, A_Wk, A_Wv, A_Wo, A_seg_len)
    x = x + _B_ref(_layernorm(x, axis=-1), B_w_r, B_w_i)
    return x
```

```python
import math

import jax
import jax.numpy as jnp
import ml_dtypes
import numpy as np
from jax.experimental import pallas as pl
from jax.experimental.pallas import tpu as pltpu

S, DM, H, DH, M, SEG = 2048, 640, 32, 128, 8, 32
L = M + SEG
NSEG = S // SEG
DF = DM // 2 + 1
G = 4
NG = H // G
F32, BF16, U32 = jnp.float32, jnp.bfloat16, jnp.uint32
C1, C2 = math.cos(2 * math.pi / 5), math.cos(4 * math.pi / 5)
S1, S2 = math.sin(2 * math.pi / 5), math.sin(4 * math.pi / 5)


def _dft_constants():
    bf = ml_dtypes.bfloat16
    d2 = np.arange(128)
    fwd = np.zeros((3, 256, 256))
    inv = np.zeros((3, 256, 256))
    scale = 1.0 / (DM * S)
    for r in range(3):
        for j in range(128 if r else 65):
            sg = -1.0 if r and j >= 64 else 1.0
            k = r + 5 * j if sg > 0 else DM - (5 - r + 5 * (j - 64))
            th = 2 * np.pi * ((d2 * k) % DM) / DM
            c, s = np.cos(th), np.sin(th)
            if k in (0, DM // 2):
                s = np.zeros(128)
            fwd[r, :128, j] = c
            fwd[r, :128, 128 + j] = -sg * s
            if r:
                fwd[r, 128:, j] = -s
                fwd[r, 128:, 128 + j] = -sg * c
            w = scale * (1.0 if k in (0, DM // 2) else 2.0)
            inv[r, j, :128] = w * c
            inv[r, 128 + j, :128] = -w * sg * s
            if r:
                inv[r, j, 128:] = w * s
                inv[r, 128 + j, 128:] = w * sg * c
    sf = np.zeros((16, 256, 256))
    for k1 in range(16):
        m = k1 + 16 * np.arange(128)
        th = 2 * np.pi * ((m[:, None] * d2[None, :]) % S) / S
        fr, fi = np.cos(th), -np.sin(th)
        sf[k1] = np.block([[fr, -fi], [fi, fr]])
    si = np.transpose(sf, (0, 2, 1))
    return (fwd.reshape(768, 256).astype(bf), inv.reshape(768, 256).astype(bf),
            sf.astype(bf), np.ascontiguousarray(si).astype(bf))


def _mm(a, b):
    return jnp.dot(a, b, preferred_element_type=F32)


def _layernorm(x):
    m = jnp.sum(x, axis=-1, keepdims=True) * (1.0 / DM)
    xc = x - m
    v = jnp.sum(xc * xc, axis=-1, keepdims=True) * (1.0 / DM)
    return xc * jax.lax.rsqrt(v + 1e-5)


def _tiles(x):
    return [x[:, i * 128:(i + 1) * 128] for i in range(x.shape[1] // 128)]


def _radix5(x):
    x0, x1, x2, x3, x4 = _tiles(x)
    a1, a2, b1, b2 = x1 + x4, x2 + x3, x1 - x4, x2 - x3
    return jnp.concatenate([x0 + a1 + a2,
                            x0 + C1 * a1 + C2 * a2, S1 * b1 + S2 * b2,
                            x0 + C2 * a1 + C1 * a2, S2 * b1 - S1 * b2], axis=1)


def _inv_radix5(t):
    t0, t1r, t1i, t2r, t2i = _tiles(t)
    a1, b1 = t0 + C1 * t1r + C2 * t2r, S1 * t1i + S2 * t2i
    a2, b2 = t0 + C2 * t1r + C1 * t2r, S2 * t1i - S1 * t2i
    return jnp.concatenate([t0 + t1r + t2r, a1 - b1, a2 - b2, a2 + b2, a1 + b1], axis=1)


def _dft4(z, sign):
    (ar, ai), (br, bi), (cr, ci), (dr, di) = z
    pr, pi, mr, mi = ar + cr, ai + ci, ar - cr, ai - ci
    qr, qi, nr, ni = br + dr, bi + di, br - dr, bi - di
    lo, hi = (mr + ni, mi - nr), (mr - ni, mi + nr)
    if sign > 0:
        lo, hi = hi, lo
    return [(pr + qr, pi + qi), lo, (pr - qr, pi - qi), hi]


def _twiddle16(z, e, sign):
    zr, zi = z
    if e == 0:
        return z
    if e == 4:
        return (-zi, zr) if sign > 0 else (zi, -zr)
    c, s = math.cos(math.pi * e / 8), sign * math.sin(math.pi * e / 8)
    if e in (2, 6):
        if c * s > 0:
            return (zr - zi) * c, (zr + zi) * c
        return (zr + zi) * c, (zi - zr) * c
    return zr * c - zi * s, zr * s + zi * c


def _dft16(z, sign):
    u = [_dft4([z[4 * a + b] for a in range(4)], sign) for b in range(4)]
    out = [None] * 16
    for c in range(4):
        v = _dft4([_twiddle16(u[b][c], b * c, sign) for b in range(4)], sign)
        for d in range(4):
            out[c + 4 * d] = v[d]
    return out


def _kernel(x_hbm, mem_ref, wq_hbm, wk_hbm, wv_hbm, wo_hbm, wr_hbm, wi_hbm,
            df_hbm, di_hbm, sf_hbm, si_hbm, out_hbm,
            io_ref, raw_ref, wo_raw, tmp_ref, w_ref, wo_ref, flt_raw, flt_ref,
            df_ref, di_ref, sf_ref, si_ref,
            x_ref, t_ref, r_ref, z_ref, u_ref, hn_ref, ao_ref, sems):
    copies = [pltpu.make_async_copy(src, dst, sems.at[i]) for i, (src, dst) in enumerate([
        (wq_hbm, raw_ref.at[0]), (wk_hbm, raw_ref.at[1]), (wv_hbm, raw_ref.at[2]),
        (wo_hbm, wo_raw), (x_hbm, io_ref),
        (wr_hbm, flt_raw.at[0]), (wi_hbm, flt_raw.at[1]),
        (df_hbm, df_ref), (di_hbm, di_ref), (sf_hbm, sf_ref), (si_hbm, si_ref)])]
    for c in copies[:5]:
        c.start()

    def rows(i, n):
        return pl.ds(pl.multiple_of(i * n, n), n)

    for i in range(3):
        copies[i].wait()

        @pl.loop(0, DM // 16)
        def _(c):
            v = raw_ref[i, rows(c, 16)].reshape(16 * H, DH)
            tmp_ref[rows(c, 8 * H), :] = pltpu.bitcast(v, U32)

        @pl.loop(0, DM // 32)
        def _(c):
            for j in range(H // 2):
                e = tmp_ref[pl.ds(c * 16 * H + j, 16, stride=H), :]
                o = tmp_ref[pl.ds(c * 16 * H + H // 2 + j, 16, stride=H), :]
                w_ref[i, rows(c, 16), 2 * j * DH:(2 * j + 1) * DH] = (e & 0xFFFF) | (o << 16)
                w_ref[i, rows(c, 16), (2 * j + 1) * DH:(2 * j + 2) * DH] = (
                    (e >> 16) | (o & np.uint32(0xFFFF0000)))

    copies[3].wait()

    @pl.loop(0, H)
    def _(c):
        wo_ref[rows(c, DH // 2), :] = pltpu.bitcast(wo_raw[rows(c, DH), :], U32)

    copies[4].wait()
    for c in copies[5:]:
        c.start()

    @pl.loop(0, S // 64)
    def _(c):
        x_ref[rows(c, 64), :] = io_ref[rows(c, 64), :].astype(F32)
        t_ref[rows(c, 64), :] = jnp.zeros((64, DM), F32)

    ao_ref[...] = jnp.zeros((SEG, DM), F32)

    def prepare_filter():
        for c in copies[5:]:
            c.wait()
        for p in range(2):
            @pl.loop(0, S // 128)
            def _(c):
                blk = pl.ds(pl.multiple_of(c * 128, 128), 128)
                tmp_ref[3 * S:3 * S + DF - 1, :] = pltpu.bitcast(flt_raw[p, :DF - 1, blk].astype(F32), U32)
                last = jnp.concatenate([flt_raw[p, DF - 1:, blk].astype(F32), jnp.zeros((63, 128), F32)], axis=0)
                part = [tmp_ref[pl.ds(3 * S + k, 64, stride=5), :] for k in range(5)]
                for r in range(3):
                    v = jnp.concatenate([part[r], part[5 - r] if r else pltpu.bitcast(last, U32)], axis=0)
                    tmp_ref[pl.ds(pl.multiple_of(r * S + c * 128, 128), 128), :] = v.T

            @pl.loop(0, 16)
            def _(k1):
                v = jnp.concatenate([tmp_ref[pl.ds(r * S + k1, 128, stride=16), :] for r in range(3)], axis=1)
                flt_ref[k1, p * 128:(p + 1) * 128, :] = pltpu.bitcast(v, F32)

    def enter(s):
        x = x_ref[rows(s, SEG), :] + _inv_radix5(t_ref[rows(s, SEG), :])
        x_ref[rows(s, SEG), :] = x
        t_ref[rows(s, SEG), :] = jnp.zeros((SEG, DM), F32)
        hn_ref[...] = _layernorm(x)

    def leave(s):
        x = x_ref[rows(s, SEG), :] + ao_ref[...]
        x_ref[rows(s, SEG), :] = x
        r_ref[rows(s, SEG), :] = _radix5(_layernorm(x)).astype(BF16)

    ri = jax.lax.broadcasted_iota(jnp.int32, (L, L), 0)
    ci = jax.lax.broadcasted_iota(jnp.int32, (L, L), 1)
    mask = (ri < M) | (ri >= ci)

    def segment(s, mem):
        h = jnp.concatenate([mem, hn_ref[...]], axis=0)
        leave(jnp.maximum(s - 1, 0))
        enter(jnp.minimum(s + 1, NSEG - 1))

        def proj(i, g):
            acc = None
            for k in range(DM // 128):
                w = w_ref[i, k * 64:(k + 1) * 64, g * G * DH:(g + 1) * G * DH]
                t = _mm(h[:, k * 128:(k + 1) * 128], pltpu.bitcast(w, BF16))
                acc = t if acc is None else acc + t
            return acc

        def scores(q, k):
            res = []
            for qh, kh in zip(_tiles(q), _tiles(k)):
                sc = jax.lax.dot_general(qh, kh.astype(BF16), (((1,), (1,)), ((), ())),
                                         preferred_element_type=F32)
                sc = jnp.where(mask, sc * DH ** -0.5, -1e9)
                e = jnp.exp(sc - jnp.max(sc, axis=-1, keepdims=True))
                d = jnp.sum(e, axis=-1, keepdims=True)
                r = pltpu.reciprocal(d, approx=True)
                res.append((e, r * (2.0 - d * r)))
            return res

        def values(es, v):
            return jnp.concatenate(
                [_mm(e, vh.astype(BF16)) * r for (e, r), vh in zip(es, _tiles(v))], axis=1)

        def project_out(o, g):
            return _mm(o, pltpu.bitcast(wo_ref[g * G * 64:(g + 1) * G * 64, :], BF16))

        os_, es, v = [], None, None
        for g in range(NG):
            q, k = proj(0, g), proj(1, g)
            if g:
                os_.append(values(es, v))
            v = proj(2, g)
            es = scores(q, k)
        out = project_out(os_[0], 0)
        for g in range(1, NG - 2):
            out = out + project_out(os_[g], g)
        os_.append(values(es, v))
        for g in range(NG - 2, NG):
            out = out + project_out(os_[g], g)
        ao_ref[...] = out[M:]
        return out[:M]

    def spectral():
        @pl.loop(0, 8)
        def _(c):
            def at(n1):
                return pl.ds(pl.multiple_of(n1 * 128 + c * 16, 16), 16)
            lhs = jnp.concatenate([r_ref[at(n1), :] for n1 in range(16)], axis=0)
            for r in range(3):
                if r == 0:
                    y = _mm(lhs[:, :128], df_ref[:128, :])
                else:
                    y = _mm(lhs[:, r * 256 - 128:r * 256 + 128], df_ref[r * 256:(r + 1) * 256, :])
                halves = [_dft16([(y[n1 * 16 + o:n1 * 16 + o + 8, :128], y[n1 * 16 + o:n1 * 16 + o + 8, 128:])
                                  for n1 in range(16)], -1) for o in (0, 8)]
                for k1 in range(16):
                    for p in range(2):
                        z_ref[k1, pl.ds(pl.multiple_of(p * 128 + c * 16, 16), 16), r * 128:(r + 1) * 128] = (
                            jnp.concatenate([halves[0][k1][p], halves[1][k1][p]], axis=0).astype(BF16))

        @pl.loop(0, 16)
        def _(k1):
            x = _mm(sf_ref[k1], z_ref[k1])
            w = flt_ref[k1]
            xr, xi, wr, wi = x[:128], x[128:], w[:128], w[128:]
            y = jnp.concatenate([xr * wr - xi * wi, xr * wi + xi * wr], axis=0).astype(BF16)
            u_ref[k1] = _mm(si_ref[k1], y)

        @pl.loop(0, 8)
        def _(c):
            for r in range(3):
                cols = slice(r * 128, (r + 1) * 128)
                halves = [_dft16([(u_ref[k1, pl.ds(pl.multiple_of(c * 16 + o, 8), 8), cols],
                                   u_ref[k1, pl.ds(pl.multiple_of(128 + c * 16 + o, 8), 8), cols])
                                  for k1 in range(16)], 1) for o in (0, 8)]
                lhs = jnp.concatenate(
                    [jnp.concatenate([hf[n1][p] for n1 in range(16) for hf in halves], axis=0)
                     for p in range(2)], axis=1).astype(BF16)
                if r == 0:
                    t, dst = _mm(lhs, di_ref[:256, :128]), slice(0, 128)
                else:
                    t, dst = _mm(lhs, di_ref[r * 256:(r + 1) * 256, :]), slice(r * 256 - 128, r * 256 + 128)
                for n1 in range(16):
                    t_ref[pl.ds(pl.multiple_of(n1 * 128 + c * 16, 16), 16), dst] = t[n1 * 16:(n1 + 1) * 16]

    @pl.loop(0, 2)
    def _(layer):
        enter(0)
        jax.lax.fori_loop(0, NSEG, segment, mem_ref[...].astype(F32))
        leave(NSEG - 1)
        ao_ref[...] = jnp.zeros((SEG, DM), F32)
        pl.when(layer == 0)(prepare_filter)
        spectral()

    outs = [pltpu.make_async_copy(io_ref.at[pl.ds(i * 256, 256)], out_hbm.at[pl.ds(i * 256, 256)],
                                  sems.at[i]) for i in range(S // 256)]
    for i, cp in enumerate(outs):
        @pl.loop(0, 4)
        def _(c):
            rs = pl.ds(pl.multiple_of(i * 256 + c * 64, 64), 64)
            io_ref[rs, :] = (x_ref[rs, :] + _inv_radix5(t_ref[rs, :])).astype(BF16)
        cp.start()
    for cp in outs:
        cp.wait()


@jax.jit
def pallas_interleave_layers__memory_aug_recurrent_mem_tr__spectral_gfnet__prompt_kernel(
    A_x: jax.Array,
    A_mem0: jax.Array,
    A_Wq: jax.Array,
    A_Wk: jax.Array,
    A_Wv: jax.Array,
    A_Wo: jax.Array,
    A_seg_len: jax.Array,
    B_x: jax.Array,
    B_w_r: jax.Array,
    B_w_i: jax.Array,
):
    del A_seg_len, B_x
    assert A_x.shape == (1, S, DM) and A_mem0.shape == (1, M, DM) and A_Wq.shape == (DM, H, DH)
    hbm = pl.BlockSpec(memory_space=pltpu.HBM)
    out = pl.pallas_call(
        _kernel,
        out_shape=jax.ShapeDtypeStruct((S, DM), BF16),
        in_specs=[hbm, pl.BlockSpec(memory_space=pltpu.VMEM)] + [hbm] * 10,
        out_specs=hbm,
        scratch_shapes=[
            pltpu.VMEM((S, DM), BF16),
            pltpu.VMEM((3, DM, H, DH), BF16),
            pltpu.VMEM((H * DH, DM), BF16),
            pltpu.VMEM((DM * H // 2, DH), U32),
            pltpu.VMEM((3, DM // 2, H * DH), U32),
            pltpu.VMEM((H * DH // 2, DM), U32),
            pltpu.VMEM((2, DF, S), BF16),
            pltpu.VMEM((16, 256, 384), F32),
            pltpu.VMEM((768, 256), BF16),
            pltpu.VMEM((768, 256), BF16),
            pltpu.VMEM((16, 256, 256), BF16),
            pltpu.VMEM((16, 256, 256), BF16),
            pltpu.VMEM((S, DM), F32),
            pltpu.VMEM((S, DM), F32),
            pltpu.VMEM((S, DM), BF16),
            pltpu.VMEM((16, 256, 384), BF16),
            pltpu.VMEM((16, 256, 384), F32),
            pltpu.VMEM((SEG, DM), F32),
            pltpu.VMEM((SEG, DM), F32),
            pltpu.SemaphoreType.DMA((12,)),
        ],
        compiler_params=pltpu.CompilerParams(vmem_limit_bytes=120 * 1024 * 1024),
    )(A_x.reshape(S, DM), A_mem0.reshape(M, DM), A_Wq, A_Wk, A_Wv, A_Wo.reshape(H * DH, DM),
      B_w_r.T, B_w_i.T, *_dft_constants())
    return out.reshape(1, S, DM)
```

```python
import math

import jax
import jax.numpy as jnp
import ml_dtypes
import numpy as np
from jax.experimental import pallas as pl
from jax.experimental.pallas import tpu as pltpu

S, DM, H, DH, M, SEG = 2048, 640, 32, 128, 8, 32
L = M + SEG
NSEG = S // SEG
DF = DM // 2 + 1
G = 4
NG = H // G
AHEAD, RING = 288, 384
WP, FP = 321, 129
F32, BF16, U32 = jnp.float32, jnp.bfloat16, jnp.uint32
C1, C2 = math.cos(2 * math.pi / 5), math.cos(4 * math.pi / 5)
S1, S2 = math.sin(2 * math.pi / 5), math.sin(4 * math.pi / 5)


def _dft_constants():
    bf = ml_dtypes.bfloat16
    d2 = np.arange(128)
    fwd = np.zeros((3, 256, 256))
    inv = np.zeros((3, 256, 256))
    scale = 1.0 / (DM * S)
    for r in range(3):
        for j in range(128 if r else 65):
            sg = -1.0 if r and j >= 64 else 1.0
            k = r + 5 * j if sg > 0 else DM - (5 - r + 5 * (j - 64))
            th = 2 * np.pi * ((d2 * k) % DM) / DM
            c, s = np.cos(th), np.sin(th)
            if k in (0, DM // 2):
                s = np.zeros(128)
            fwd[r, :128, j] = c
            fwd[r, :128, 128 + j] = -sg * s
            if r:
                fwd[r, 128:, j] = -s
                fwd[r, 128:, 128 + j] = -sg * c
            w = scale * (1.0 if k in (0, DM // 2) else 2.0)
            inv[r, j, :128] = w * c
            inv[r, 128 + j, :128] = -w * sg * s
            if r:
                inv[r, j, 128:] = w * s
                inv[r, 128 + j, 128:] = w * sg * c
    sf = np.zeros((16, 256, 256))
    for k1 in range(16):
        m = k1 + 16 * np.arange(128)
        th = 2 * np.pi * ((m[:, None] * d2[None, :]) % S) / S
        fr, fi = np.cos(th), -np.sin(th)
        sf[k1] = np.block([[fr, -fi], [fi, fr]])
    si = np.transpose(sf, (0, 2, 1))
    return (fwd.reshape(768, 256).astype(bf), inv.reshape(768, 256).astype(bf),
            sf.astype(bf), np.ascontiguousarray(si).astype(bf))


def _mm(a, b):
    return jnp.dot(a, b, preferred_element_type=F32)


def _layernorm(x):
    m = jnp.sum(x, axis=-1, keepdims=True) * (1.0 / DM)
    xc = x - m
    v = jnp.sum(xc * xc, axis=-1, keepdims=True) * (1.0 / DM)
    return xc * jax.lax.rsqrt(v + 1e-5)


def _tiles(x):
    return [x[:, i * 128:(i + 1) * 128] for i in range(x.shape[1] // 128)]


def _radix5(x):
    x0, x1, x2, x3, x4 = _tiles(x)
    a1, a2, b1, b2 = x1 + x4, x2 + x3, x1 - x4, x2 - x3
    return jnp.concatenate([x0 + a1 + a2,
                            x0 + C1 * a1 + C2 * a2, S1 * b1 + S2 * b2,
                            x0 + C2 * a1 + C1 * a2, S2 * b1 - S1 * b2], axis=1)


def _inv_radix5(t):
    t0, t1r, t1i, t2r, t2i = _tiles(t)
    a1, b1 = t0 + C1 * t1r + C2 * t2r, S1 * t1i + S2 * t2i
    a2, b2 = t0 + C2 * t1r + C1 * t2r, S2 * t1i - S1 * t2i
    return jnp.concatenate([t0 + t1r + t2r, a1 - b1, a2 - b2, a2 + b2, a1 + b1], axis=1)


def _dft4(z, sign):
    (ar, ai), (br, bi), (cr, ci), (dr, di) = z
    pr, pi, mr, mi = ar + cr, ai + ci, ar - cr, ai - ci
    qr, qi, nr, ni = br + dr, bi + di, br - dr, bi - di
    lo, hi = (mr + ni, mi - nr), (mr - ni, mi + nr)
    if sign > 0:
        lo, hi = hi, lo
    return [(pr + qr, pi + qi), lo, (pr - qr, pi - qi), hi]


def _twiddle16(z, e, sign):
    zr, zi = z
    if e == 0:
        return z
    if e == 4:
        return (-zi, zr) if sign > 0 else (zi, -zr)
    c, s = math.cos(math.pi * e / 8), sign * math.sin(math.pi * e / 8)
    if e in (2, 6):
        if c * s > 0:
            return (zr - zi) * c, (zr + zi) * c
        return (zr + zi) * c, (zi - zr) * c
    return zr * c - zi * s, zr * s + zi * c


def _dft16(z, sign):
    u = [_dft4([z[4 * a + b] for a in range(4)], sign) for b in range(4)]
    out = [None] * 16
    for c in range(4):
        v = _dft4([_twiddle16(u[b][c], b * c, sign) for b in range(4)], sign)
        for d in range(4):
            out[c + 4 * d] = v[d]
    return out


def _kernel(x_hbm, mem_ref, wq_hbm, wk_hbm, wv_hbm, wo_hbm, wr_hbm, wi_hbm,
            df_hbm, di_hbm, sf_hbm, si_hbm, out_hbm,
            io_ref, raw_ref, w_ref, wo_ref, flt_raw, tmp_ref, flt_ref,
            df_ref, di_ref, sf_ref, si_ref,
            x_ref, t_ref, r_ref, z_ref, u_ref, hn_ref, ao_ref, hb_ref, qkv_ref, sems):
    halves = [(i, j) for i in range(3) for j in range(2)]
    head, rest = pl.ds(0, AHEAD), pl.ds(AHEAD, S - AHEAD)
    copies = [pltpu.make_async_copy(src, dst, sems.at[i]) for i, (src, dst) in enumerate(
        [((wq_hbm, wk_hbm, wv_hbm)[i].at[:, pl.ds(16 * j, 16), :], raw_ref.at[2 * i + j]) for i, j in halves]
        + [(x_hbm.at[rest], io_ref.at[rest]), (wo_hbm, wo_ref),
           (wr_hbm, flt_raw.at[0]), (wi_hbm, flt_raw.at[1]),
           (df_hbm, df_ref), (di_hbm, di_ref), (sf_hbm, sf_ref), (si_hbm, si_ref),
           (x_hbm.at[head], io_ref.at[head])])]

    def rows(i, n):
        return pl.ds(pl.multiple_of(i * n, n), n)

    def weights(i, g, k):
        tiles = []
        for hd in range(g * G, (g + 1) * G):
            start = ((2 * i + hd // 16) * 16 + hd % 2 * 8 + hd % 16 // 2) * WP + k * 64
            tiles.append(w_ref[start:start + 64, :])
        return pltpu.bitcast(jnp.concatenate(tiles, axis=1), BF16)

    def project(h, i, g):
        acc = None
        for k in range(DM // 128):
            t = _mm(h[:, k * 128:(k + 1) * 128], weights(i, g, k))
            acc = t if acc is None else acc + t
        return acc

    def load_rows(c):
        x = io_ref[rows(c, SEG), :].astype(F32)
        x_ref[rows(c, SEG), :] = x
        return x

    copies[14].start()
    copies[0].start()
    flt_raw[2, :, :128] = jnp.zeros((DF, 128), BF16)
    ao_ref[...] = jnp.zeros((SEG, DM), F32)
    copies[14].wait()
    copies[1].start()

    @pl.loop(0, AHEAD // SEG)
    def _(c):
        hb_ref[rows(c, SEG), :] = _layernorm(load_rows(c)).astype(BF16)

    for n, (i, j) in enumerate(halves):
        copies[n].wait()
        copies[n + 2].start()

        @pl.loop(0, DM // 32)
        def _(c):
            v = pltpu.bitcast(raw_ref[n, rows(c, 32)].reshape(32 * 16, DH), U32)
            for q in range(16):
                e, o = v[16 * q:16 * q + 8], v[16 * q + 8:16 * q + 16]
                at = n * 16 * WP + c * 16 + q
                w_ref[pl.ds(at, 8, stride=WP), :] = (e & 0xFFFF) | (o << 16)
                w_ref[pl.ds(at + 8 * WP, 8, stride=WP), :] = (e >> 16) | (o & np.uint32(0xFFFF0000))

        if n == 5:
            copies[6].wait()

        @pl.loop(0, AHEAD // 96)
        def _(c):
            for g in range(j * NG // 2, (j + 1) * NG // 2):
                qkv_ref[i, rows(c, 96), g * G * DH:(g + 1) * G * DH] = project(hb_ref[rows(c, 96), :], i, g)
            if n == 5:
                per = -(-(NSEG - AHEAD // SEG) // (AHEAD // 96))
                for q in range(per):
                    load_rows(jnp.minimum(AHEAD // SEG + c * per + q, NSEG - 1))

    copies[7].wait()
    for c in copies[8:14]:
        c.start()

    def prepare_filter(p, c):
        blk = pl.ds(pl.multiple_of(c * 128, 128), 128)
        tmp_ref[...] = flt_raw[p, :DF - 1, blk].astype(F32)
        last = jnp.concatenate([flt_raw[p, DF - 1:, blk].astype(F32), jnp.zeros((63, 128), F32)], axis=0)
        part = [tmp_ref[pl.ds(k, 64, stride=5), :] for k in range(5)]
        for r in range(3):
            v = jnp.concatenate([part[r], part[5 - r] if r else last], axis=0).T
            for q in range(16):
                at = ((p % 2 * 3 + r) * 16 + q % 2 * 8) * FP + c * 8 + q // 2
                flt_ref[pl.ds(at, 8, stride=FP), :] = v[8 * q:8 * q + 8]

    def enter(rs, layer):
        x = x_ref[rs, :]
        if layer is not None:
            x = x + jnp.where(layer > 0, _inv_radix5(t_ref[rs, :]), 0.0)
            x_ref[rs, :] = x
            t_ref[rs, :] = jnp.zeros((SEG, DM), F32)
        hn_ref[...] = _layernorm(x)

    def leave(s):
        x = x_ref[rows(s, SEG), :] + ao_ref[...]
        x_ref[rows(s, SEG), :] = x
        r_ref[rows(s, SEG), :] = _radix5(_layernorm(x)).astype(BF16)

    ri = jax.lax.broadcasted_iota(jnp.int32, (L, L), 0)
    ci = jax.lax.broadcasted_iota(jnp.int32, (L, L), 1)
    mask = (ri < M) | (ri >= ci)

    def segment(s, mem, layer):
        early = layer is None
        if early:
            @pl.when(s == 2)
            def _():
                copies[8].wait()
                copies[9].wait()

        h = jnp.concatenate([mem, hn_ref[:SEG - M if early else SEG, :]], axis=0)
        leave(jnp.maximum(s - 1, 0))
        if early:
            enter(pl.ds(pl.multiple_of(AHEAD + (s + 1) * (SEG - M), 8), SEG), None)
            piece = jnp.clip(s - 2, 0, 31)
            prepare_filter(jnp.where(s < 2, 2, piece // 16), piece % 16)
            put = pl.ds(pl.multiple_of((AHEAD + s * (SEG - M)) % RING, 8), SEG - M)
            get = pl.ds(pl.multiple_of(s * SEG % RING, SEG), SEG)
        else:
            enter(rows(jnp.minimum(s + 1, NSEG - 1), SEG), layer)

        def proj(i, g):
            y = project(h, i, g)
            if early:
                cols = slice(g * G * DH, (g + 1) * G * DH)
                qkv_ref[i, put, cols] = y[M:]
                y = jnp.concatenate([y[:M], qkv_ref[i, get, cols]], axis=0)
            return y

        def scores(q, k):
            res = []
            for qh, kh in zip(_tiles(q), _tiles(k)):
                sc = jax.lax.dot_general(qh, kh.astype(BF16), (((1,), (1,)), ((), ())),
                                         preferred_element_type=F32)
                sc = jnp.where(mask, sc * DH ** -0.5, -1e9)
                e = jnp.exp(sc - jnp.max(sc, axis=-1, keepdims=True))
                d = jnp.sum(e, axis=-1, keepdims=True)
                r = pltpu.reciprocal(d, approx=True)
                res.append((e, r * (2.0 - d * r)))
            return res

        def values(es, v):
            return jnp.concatenate(
                [_mm(e, vh.astype(BF16)) * r for (e, r), vh in zip(es, _tiles(v))], axis=1)

        def project_out(o, g):
            return _mm(o, wo_ref[g * G * DH:(g + 1) * G * DH, :])

        os_, es, v = [], None, None
        for g in range(NG):
            q, k = proj(0, g), proj(1, g)
            if g:
                os_.append(values(es, v))
            v = proj(2, g)
            es = scores(q, k)
        out = project_out(os_[0], 0)
        for g in range(1, NG - 2):
            out = out + project_out(os_[g], g)
        os_.append(values(es, v))
        for g in range(NG - 2, NG):
            out = out + project_out(os_[g], g)
        ao_ref[...] = out[M:]
        return out[:M]

    def spectral():
        @pl.loop(0, 8)
        def _(c):
            def at(n1):
                return pl.ds(pl.multiple_of(n1 * 128 + c * 16, 16), 16)
            lhs = jnp.concatenate([r_ref[at(n1), :] for n1 in range(16)], axis=0)
            for r in range(3):
                if r == 0:
                    y = _mm(lhs[:, :128], df_ref[:128, :])
                else:
                    y = _mm(lhs[:, r * 256 - 128:r * 256 + 128], df_ref[r * 256:(r + 1) * 256, :])
                parts = [_dft16([(y[n1 * 16 + o:n1 * 16 + o + 8, :128], y[n1 * 16 + o:n1 * 16 + o + 8, 128:])
                                  for n1 in range(16)], -1) for o in (0, 8)]
                for k1 in range(16):
                    for p in range(2):
                        z_ref[k1, pl.ds(pl.multiple_of(p * 128 + c * 16, 16), 16), r * 128:(r + 1) * 128] = (
                            jnp.concatenate([parts[0][k1][p], parts[1][k1][p]], axis=0).astype(BF16))

        @pl.loop(0, 16)
        def _(k1):
            x = _mm(sf_ref[k1], z_ref[k1])
            wr, wi = (jnp.concatenate([flt_ref[pl.ds(((p * 3 + r) * 16 + k1) * FP, 128), :]
                                       for r in range(3)], axis=1) for p in range(2))
            xr, xi = x[:128], x[128:]
            y = jnp.concatenate([xr * wr - xi * wi, xr * wi + xi * wr], axis=0).astype(BF16)
            u_ref[k1] = _mm(si_ref[k1], y)

        @pl.loop(0, 8)
        def _(c):
            for r in range(3):
                cols = slice(r * 128, (r + 1) * 128)
                parts = [_dft16([(u_ref[k1, pl.ds(pl.multiple_of(c * 16 + o, 8), 8), cols],
                                   u_ref[k1, pl.ds(pl.multiple_of(128 + c * 16 + o, 8), 8), cols])
                                  for k1 in range(16)], 1) for o in (0, 8)]
                lhs = jnp.concatenate(
                    [jnp.concatenate([hf[n1][p] for n1 in range(16) for hf in parts], axis=0)
                     for p in range(2)], axis=1).astype(BF16)
                if r == 0:
                    t, dst = _mm(lhs, di_ref[:256, :128]), slice(0, 128)
                else:
                    t, dst = _mm(lhs, di_ref[r * 256:(r + 1) * 256, :]), slice(r * 256 - 128, r * 256 + 128)
                for n1 in range(16):
                    t_ref[pl.ds(pl.multiple_of(n1 * 128 + c * 16, 16), 16), dst] = t[n1 * 16:(n1 + 1) * 16]

    mem0 = mem_ref[...].astype(F32)
    enter(pl.ds(AHEAD, SEG), None)
    mem1 = jax.lax.fori_loop(0, AHEAD // M, lambda s, m: segment(s, m, None), mem0)
    for c in copies[10:14]:
        c.wait()

    @pl.loop(0, 2)
    def _(layer):
        first = jnp.where(layer == 0, AHEAD // M, 0)
        enter(rows(first, SEG), layer)
        jax.lax.fori_loop(first, NSEG, lambda s, m: segment(s, m, layer), jnp.where(layer == 0, mem1, mem0))
        leave(NSEG - 1)
        ao_ref[...] = jnp.zeros((SEG, DM), F32)
        spectral()

    outs = [pltpu.make_async_copy(io_ref.at[pl.ds(i * 256, 256)], out_hbm.at[pl.ds(i * 256, 256)],
                                  sems.at[i]) for i in range(S // 256)]
    for i, cp in enumerate(outs):
        @pl.loop(0, 4)
        def _(c):
            rs = pl.ds(pl.multiple_of(i * 256 + c * 64, 64), 64)
            io_ref[rs, :] = (x_ref[rs, :] + _inv_radix5(t_ref[rs, :])).astype(BF16)
        cp.start()
    for cp in outs:
        cp.wait()


@jax.jit
def pallas_interleave_layers__memory_aug_recurrent_mem_tr__spectral_gfnet__prompt_kernel(
    A_x: jax.Array,
    A_mem0: jax.Array,
    A_Wq: jax.Array,
    A_Wk: jax.Array,
    A_Wv: jax.Array,
    A_Wo: jax.Array,
    A_seg_len: jax.Array,
    B_x: jax.Array,
    B_w_r: jax.Array,
    B_w_i: jax.Array,
):
    del A_seg_len, B_x
    assert A_x.shape == (1, S, DM) and A_mem0.shape == (1, M, DM) and A_Wq.shape == (DM, H, DH)
    hbm = pl.BlockSpec(memory_space=pltpu.HBM)
    out = pl.pallas_call(
        _kernel,
        out_shape=jax.ShapeDtypeStruct((S, DM), BF16),
        in_specs=[hbm, pl.BlockSpec(memory_space=pltpu.VMEM)] + [hbm] * 10,
        out_specs=hbm,
        scratch_shapes=[
            pltpu.VMEM((S, DM), BF16),
            pltpu.VMEM((6, DM, 16, DH), BF16),
            pltpu.VMEM((3 * H * WP, DH), U32),
            pltpu.VMEM((H * DH, DM), BF16),
            pltpu.VMEM((3, DF, S), BF16),
            pltpu.VMEM((DF - 1, 128), F32),
            pltpu.VMEM((6 * 16 * FP, 128), F32),
            pltpu.VMEM((768, 256), BF16),
            pltpu.VMEM((768, 256), BF16),
            pltpu.VMEM((16, 256, 256), BF16),
            pltpu.VMEM((16, 256, 256), BF16),
            pltpu.VMEM((S, DM), F32),
            pltpu.VMEM((S, DM), F32),
            pltpu.VMEM((S, DM), BF16),
            pltpu.VMEM((16, 256, 384), BF16),
            pltpu.VMEM((16, 256, 384), F32),
            pltpu.VMEM((SEG, DM), F32),
            pltpu.VMEM((SEG, DM), F32),
            pltpu.VMEM((AHEAD, DM), BF16),
            pltpu.VMEM((3, RING, H * DH), F32),
            pltpu.SemaphoreType.DMA((15,)),
        ],
        compiler_params=pltpu.CompilerParams(vmem_limit_bytes=120 * 1024 * 1024),
    )(A_x.reshape(S, DM), A_mem0.reshape(M, DM), A_Wq, A_Wk, A_Wv, A_Wo.reshape(H * DH, DM),
      B_w_r.T, B_w_i.T, *_dft_constants())
    return out.reshape(1, S, DM)
```

```python
import math

import jax
import jax.numpy as jnp
import ml_dtypes
import numpy as np
from jax.experimental import pallas as pl
from jax.experimental.pallas import tpu as pltpu

S, DM, H, DH, M, SEG = 2048, 640, 32, 128, 8, 32
L = M + SEG
NSEG = S // SEG
DF = DM // 2 + 1
G = 4
NG = H // G
AHEAD, RING = 288, 384
UNROLL, CU, KU = 2, 2, 8
WP, FP = 321, 129
F32, BF16, U32 = jnp.float32, jnp.bfloat16, jnp.uint32
C1, C2 = math.cos(2 * math.pi / 5), math.cos(4 * math.pi / 5)
S1, S2 = math.sin(2 * math.pi / 5), math.sin(4 * math.pi / 5)


def _dft_constants():
    bf = ml_dtypes.bfloat16
    d2 = np.arange(128)
    fwd = np.zeros((3, 256, 256))
    inv = np.zeros((3, 256, 256))
    scale = 1.0 / (DM * S)
    for r in range(3):
        for j in range(128 if r else 65):
            sg = -1.0 if r and j >= 64 else 1.0
            k = r + 5 * j if sg > 0 else DM - (5 - r + 5 * (j - 64))
            th = 2 * np.pi * ((d2 * k) % DM) / DM
            c, s = np.cos(th), np.sin(th)
            if k in (0, DM // 2):
                s = np.zeros(128)
            fwd[r, :128, j] = c
            fwd[r, :128, 128 + j] = -sg * s
            if r:
                fwd[r, 128:, j] = -s
                fwd[r, 128:, 128 + j] = -sg * c
            w = scale * (1.0 if k in (0, DM // 2) else 2.0)
            inv[r, j, :128] = w * c
            inv[r, 128 + j, :128] = -w * sg * s
            if r:
                inv[r, j, 128:] = w * s
                inv[r, 128 + j, 128:] = w * sg * c
    sf = np.zeros((16, 256, 256))
    for k1 in range(16):
        m = k1 + 16 * np.arange(128)
        th = 2 * np.pi * ((m[:, None] * d2[None, :]) % S) / S
        fr, fi = np.cos(th), -np.sin(th)
        sf[k1] = np.block([[fr, -fi], [fi, fr]])
    si = np.transpose(sf, (0, 2, 1))
    return (fwd.reshape(768, 256).astype(bf), inv.reshape(768, 256).astype(bf),
            sf.astype(bf), np.ascontiguousarray(si).astype(bf))


def _mm(a, b):
    return jnp.dot(a, b, preferred_element_type=F32)


def _layernorm(x):
    m = jnp.sum(x, axis=-1, keepdims=True) * (1.0 / DM)
    xc = x - m
    v = jnp.sum(xc * xc, axis=-1, keepdims=True) * (1.0 / DM)
    return xc * jax.lax.rsqrt(v + 1e-5)


def _tiles(x):
    return [x[:, i * 128:(i + 1) * 128] for i in range(x.shape[1] // 128)]


def _radix5(x):
    x0, x1, x2, x3, x4 = _tiles(x)
    a1, a2, b1, b2 = x1 + x4, x2 + x3, x1 - x4, x2 - x3
    return jnp.concatenate([x0 + a1 + a2,
                            x0 + C1 * a1 + C2 * a2, S1 * b1 + S2 * b2,
                            x0 + C2 * a1 + C1 * a2, S2 * b1 - S1 * b2], axis=1)


def _inv_radix5(t):
    t0, t1r, t1i, t2r, t2i = _tiles(t)
    a1, b1 = t0 + C1 * t1r + C2 * t2r, S1 * t1i + S2 * t2i
    a2, b2 = t0 + C2 * t1r + C1 * t2r, S2 * t1i - S1 * t2i
    return jnp.concatenate([t0 + t1r + t2r, a1 - b1, a2 - b2, a2 + b2, a1 + b1], axis=1)


def _dft4(z, sign):
    (ar, ai), (br, bi), (cr, ci), (dr, di) = z
    pr, pi, mr, mi = ar + cr, ai + ci, ar - cr, ai - ci
    qr, qi, nr, ni = br + dr, bi + di, br - dr, bi - di
    lo, hi = (mr + ni, mi - nr), (mr - ni, mi + nr)
    if sign > 0:
        lo, hi = hi, lo
    return [(pr + qr, pi + qi), lo, (pr - qr, pi - qi), hi]


def _twiddle16(z, e, sign):
    zr, zi = z
    if e == 0:
        return z
    if e == 4:
        return (-zi, zr) if sign > 0 else (zi, -zr)
    c, s = math.cos(math.pi * e / 8), sign * math.sin(math.pi * e / 8)
    if e in (2, 6):
        if c * s > 0:
            return (zr - zi) * c, (zr + zi) * c
        return (zr + zi) * c, (zi - zr) * c
    return zr * c - zi * s, zr * s + zi * c


def _dft16(z, sign):
    u = [_dft4([z[4 * a + b] for a in range(4)], sign) for b in range(4)]
    out = [None] * 16
    for c in range(4):
        v = _dft4([_twiddle16(u[b][c], b * c, sign) for b in range(4)], sign)
        for d in range(4):
            out[c + 4 * d] = v[d]
    return out


def _kernel(x_hbm, mem_ref, wq_hbm, wk_hbm, wv_hbm, wo_hbm, wr_hbm, wi_hbm,
            df_hbm, di_hbm, sf_hbm, si_hbm, out_hbm,
            io_ref, raw_ref, w_ref, wo_ref, flt_raw, tmp_ref, flt_ref,
            df_ref, di_ref, sf_ref, si_ref,
            x_ref, in_ref, r_ref, z_ref, u_ref, hn_ref, ao_ref, hb_ref, qkv_ref, sems):
    halves = [(i, j) for i in range(3) for j in range(2)]
    head, rest = pl.ds(0, AHEAD), pl.ds(AHEAD, S - AHEAD)
    copies = [pltpu.make_async_copy(src, dst, sems.at[i]) for i, (src, dst) in enumerate(
        [((wq_hbm, wk_hbm, wv_hbm)[i].at[:, pl.ds(16 * j, 16), :], raw_ref.at[2 * i + j]) for i, j in halves]
        + [(x_hbm.at[rest], in_ref.at[rest]), (wo_hbm, wo_ref),
           (wr_hbm, flt_raw.at[0]), (wi_hbm, flt_raw.at[1]),
           (df_hbm, df_ref), (di_hbm, di_ref), (sf_hbm, sf_ref), (si_hbm, si_ref),
           (x_hbm.at[head], in_ref.at[head])])]

    def rows(i, n):
        return pl.ds(pl.multiple_of(i * n, n), n)

    def weights(i, g, k):
        tiles = []
        for hd in range(g * G, (g + 1) * G):
            start = ((2 * i + hd // 16) * 16 + hd % 2 * 8 + hd % 16 // 2) * WP + k * 64
            tiles.append(w_ref[start:start + 64, :])
        return pltpu.bitcast(jnp.concatenate(tiles, axis=1), BF16)

    def project(h, i, g):
        acc = None
        for k in range(DM // 128):
            t = _mm(h[:, k * 128:(k + 1) * 128], weights(i, g, k))
            acc = t if acc is None else acc + t
        return acc

    def load_rows(c):
        x = in_ref[rows(c, SEG), :].astype(F32)
        x_ref[rows(c, SEG), :] = x
        return x

    copies[14].start()
    copies[0].start()
    flt_raw[2, :, :128] = jnp.zeros((DF, 128), BF16)
    ao_ref[...] = jnp.zeros((SEG, DM), F32)
    copies[14].wait()
    copies[1].start()

    @pl.loop(0, AHEAD // SEG)
    def _(c):
        hb_ref[rows(c, SEG), :] = _layernorm(load_rows(c)).astype(BF16)

    for n, (i, j) in enumerate(halves):
        copies[n].wait()
        if n < 3:
            copies[2 * n + 2].start()
            copies[2 * n + 3].start()

        @pl.loop(0, DM // 32)
        def _(c):
            v = pltpu.bitcast(raw_ref[n, rows(c, 32)].reshape(32 * 16, DH), U32)
            for q in range(16):
                e, o = v[16 * q:16 * q + 8], v[16 * q + 8:16 * q + 16]
                at = n * 16 * WP + c * 16 + q
                w_ref[pl.ds(at, 8, stride=WP), :] = (e & 0xFFFF) | (o << 16)
                w_ref[pl.ds(at + 8 * WP, 8, stride=WP), :] = (e >> 16) | (o & np.uint32(0xFFFF0000))

        if n == 5:
            copies[6].wait()

        @pl.loop(0, AHEAD // 96)
        def _(c):
            for g in range(j * NG // 2, (j + 1) * NG // 2):
                qkv_ref[i, rows(c, 96), g * G * DH:(g + 1) * G * DH] = project(hb_ref[rows(c, 96), :], i, g)
            if n == 5:
                per = -(-(NSEG - AHEAD // SEG) // (AHEAD // 96))
                for q in range(per):
                    load_rows(jnp.minimum(AHEAD // SEG + c * per + q, NSEG - 1))

    copies[7].wait()
    for c in copies[8:14]:
        c.start()

    def prepare_filter(p, c):
        blk = pl.ds(pl.multiple_of(c * 128, 128), 128)
        tmp_ref[...] = flt_raw[p, :DF - 1, blk].astype(F32)
        last = jnp.concatenate([flt_raw[p, DF - 1:, blk].astype(F32), jnp.zeros((63, 128), F32)], axis=0)
        part = [tmp_ref[pl.ds(k, 64, stride=5), :] for k in range(5)]
        for r in range(3):
            v = jnp.concatenate([part[r], part[5 - r] if r else last], axis=0).T
            for q in range(16):
                at = ((p % 2 * 3 + r) * 16 + q % 2 * 8) * FP + c * 8 + q // 2
                flt_ref[pl.ds(at, 8, stride=FP), :] = v[8 * q:8 * q + 8]

    def enter(rs):
        hn_ref[...] = _layernorm(x_ref[rs, :])

    def leave(s):
        x = x_ref[rows(s, SEG), :] + ao_ref[...]
        x_ref[rows(s, SEG), :] = x
        r_ref[rows(s, SEG), :] = _radix5(_layernorm(x)).astype(BF16)

    ri = jax.lax.broadcasted_iota(jnp.int32, (L, L), 0)
    ci = jax.lax.broadcasted_iota(jnp.int32, (L, L), 1)
    mask = (ri < M) | (ri >= ci)

    def segment(s, mem, early):
        h = jnp.concatenate([mem, hn_ref[:SEG - M if early else SEG, :]], axis=0)
        leave(jnp.maximum(s - 1, 0))
        if early:
            enter(pl.ds(pl.multiple_of(AHEAD + (s + 1) * (SEG - M), 8), SEG))
            piece = jnp.clip(s - 4, 0, 31)
            prepare_filter(jnp.where(s < 4, 2, piece // 16), piece % 16)
            put = pl.ds(pl.multiple_of((AHEAD + s * (SEG - M)) % RING, 8), SEG - M)
            get = pl.ds(pl.multiple_of(s * SEG % RING, SEG), SEG)
        else:
            enter(rows(jnp.minimum(s + 1, NSEG - 1), SEG))

        def proj(i, g):
            y = project(h, i, g)
            if early:
                cols = slice(g * G * DH, (g + 1) * G * DH)
                qkv_ref[i, put, cols] = y[M:]
                y = jnp.concatenate([y[:M], qkv_ref[i, get, cols]], axis=0)
            return y

        def scores(q, k):
            res = []
            for qh, kh in zip(_tiles(q), _tiles(k)):
                sc = jax.lax.dot_general(qh, kh.astype(BF16), (((1,), (1,)), ((), ())),
                                         preferred_element_type=F32)
                sc = jnp.where(mask, sc * DH ** -0.5, -1e9)
                e = jnp.exp(sc - jnp.max(sc, axis=-1, keepdims=True))
                d = jnp.sum(e, axis=-1, keepdims=True)
                r = pltpu.reciprocal(d, approx=True)
                res.append((e, r * (2.0 - d * r)))
            return res

        def values(es, v):
            return jnp.concatenate(
                [_mm(e, vh.astype(BF16)) * r for (e, r), vh in zip(es, _tiles(v))], axis=1)

        def project_out(o, g):
            return _mm(o, wo_ref[g * G * DH:(g + 1) * G * DH, :])

        os_, es, v = [], None, None
        for g in range(NG):
            q, k = proj(0, g), proj(1, g)
            if g:
                os_.append(values(es, v))
            v = proj(2, g)
            es = scores(q, k)
        out = project_out(os_[0], 0)
        for g in range(1, NG - 2):
            out = out + project_out(os_[g], g)
        os_.append(values(es, v))
        for g in range(NG - 2, NG):
            out = out + project_out(os_[g], g)
        ao_ref[...] = out[M:]
        return out[:M]

    def segments(first, last, mem, early):
        def body(i, mem):
            if early:
                @pl.when(i == 4 // UNROLL)
                def _():
                    copies[8].wait()
                    copies[9].wait()
            for q in range(UNROLL):
                mem = segment(i * UNROLL + q, mem, early)
            return mem
        return jax.lax.fori_loop(first // UNROLL, last // UNROLL, body, mem)

    def out_copy(c):
        rs = pl.ds(pl.multiple_of(c * 16 * CU, 16 * CU), 16 * CU)
        return pltpu.make_async_copy(io_ref.at[:, rs, :], out_hbm.at[:, rs, :], sems.at[c])

    def spectral(layer):
        @pl.loop(0, 8, unroll=CU)
        def _(c):
            def at(n1):
                return pl.ds(pl.multiple_of(n1 * 128 + c * 16, 16), 16)
            for r in (1, 2, 0):
                src = slice(r * 256 - 128, r * 256 + 128) if r else slice(0, 128)
                lhs = jnp.concatenate([r_ref[at(n1), src] for n1 in range(16)], axis=0)
                y = _mm(lhs, df_ref[r * 256:r * 256 + lhs.shape[1], :])
                parts = [_dft16([(y[n1 * 16 + o:n1 * 16 + o + 8, :128], y[n1 * 16 + o:n1 * 16 + o + 8, 128:])
                                 for n1 in range(16)], -1) for o in (0, 8)]
                for k1 in range(16):
                    for p in range(2):
                        v = jnp.concatenate([parts[0][k1][p], parts[1][k1][p]], axis=0).astype(BF16)
                        z_ref[k1, pl.ds(pl.multiple_of(p * 64 + c * 8, 8), 8), r * 128:(r + 1) * 128] = (
                            pltpu.bitcast(v, U32))

        @pl.loop(0, 16 // KU)
        def _(i):
            ys = []
            for q in range(KU + 2):
                if q < KU:
                    k1 = i * KU + q
                    x = _mm(sf_ref[k1], pltpu.bitcast(z_ref[k1], BF16))
                    wr, wi = (jnp.concatenate([flt_ref[pl.ds(((p * 3 + r) * 16 + k1) * FP, 128), :]
                                               for r in range(3)], axis=1) for p in range(2))
                    xr, xi = x[:128], x[128:]
                    ys.append(jnp.concatenate([xr * wr - xi * wi, xr * wi + xi * wr], axis=0).astype(BF16))
                if q >= 2:
                    u_ref[i * KU + q - 2] = _mm(si_ref[i * KU + q - 2], ys[q - 2])

        @pl.loop(0, 8 // CU)
        def _(i):
            for q in range(CU):
                c = i * CU + q
                ts = []
                for r in range(3):
                    cols = slice(r * 128, (r + 1) * 128)
                    parts = [_dft16([(u_ref[k1, pl.ds(pl.multiple_of(c * 16 + o, 8), 8), cols],
                                      u_ref[k1, pl.ds(pl.multiple_of(128 + c * 16 + o, 8), 8), cols])
                                     for k1 in range(16)], 1) for o in (0, 8)]
                    lhs = jnp.concatenate(
                        [jnp.concatenate([hf[n1][p] for n1 in range(16) for hf in parts], axis=0)
                         for p in range(2)], axis=1).astype(BF16)
                    ts.append(_mm(lhs, di_ref[r * 256:(r + 1) * 256, :256 if r else 128]))
                for n1 in range(16):
                    rs = pl.ds(pl.multiple_of(n1 * 128 + c * 16, 16), 16)
                    x = x_ref[rs, :] + _inv_radix5(jnp.concatenate([t[n1 * 16:(n1 + 1) * 16] for t in ts], axis=1))
                    x_ref[rs, :] = x
                    io_ref[n1, rows(c, 16), :] = x.astype(BF16)
            pl.when(layer == 1)(lambda: out_copy(i).start())

    mem0 = mem_ref[...].astype(F32)
    enter(pl.ds(AHEAD, SEG))
    mem1 = segments(0, AHEAD // M, mem0, True)
    for c in copies[10:14]:
        c.wait()

    @pl.loop(0, 2)
    def _(layer):
        first = jnp.where(layer == 0, AHEAD // M, 0)
        enter(rows(first, SEG))
        segments(first, NSEG, jnp.where(layer == 0, mem1, mem0), False)
        leave(NSEG - 1)
        ao_ref[...] = jnp.zeros((SEG, DM), F32)
        spectral(layer)

    for i in range(8 // CU):
        out_copy(i).wait()


@jax.jit
def pallas_interleave_layers__memory_aug_recurrent_mem_tr__spectral_gfnet__prompt_kernel(
    A_x: jax.Array,
    A_mem0: jax.Array,
    A_Wq: jax.Array,
    A_Wk: jax.Array,
    A_Wv: jax.Array,
    A_Wo: jax.Array,
    A_seg_len: jax.Array,
    B_x: jax.Array,
    B_w_r: jax.Array,
    B_w_i: jax.Array,
):
    del A_seg_len, B_x
    assert A_x.shape == (1, S, DM) and A_mem0.shape == (1, M, DM) and A_Wq.shape == (DM, H, DH)
    hbm = pl.BlockSpec(memory_space=pltpu.HBM)
    out = pl.pallas_call(
        _kernel,
        out_shape=jax.ShapeDtypeStruct((16, 128, DM), BF16),
        in_specs=[hbm, pl.BlockSpec(memory_space=pltpu.VMEM)] + [hbm] * 10,
        out_specs=hbm,
        scratch_shapes=[
            pltpu.VMEM((16, 128, DM), BF16),
            pltpu.VMEM((6, DM, 16, DH), BF16),
            pltpu.VMEM((3 * H * WP, DH), U32),
            pltpu.VMEM((H * DH, DM), BF16),
            pltpu.VMEM((3, DF, S), BF16),
            pltpu.VMEM((DF - 1, 128), F32),
            pltpu.VMEM((6 * 16 * FP, 128), F32),
            pltpu.VMEM((768, 256), BF16),
            pltpu.VMEM((768, 256), BF16),
            pltpu.VMEM((16, 256, 256), BF16),
            pltpu.VMEM((16, 256, 256), BF16),
            pltpu.VMEM((S, DM), F32),
            pltpu.VMEM((S, DM), BF16),
            pltpu.VMEM((S, DM), BF16),
            pltpu.VMEM((16, 128, 384), U32),
            pltpu.VMEM((16, 256, 384), F32),
            pltpu.VMEM((SEG, DM), F32),
            pltpu.VMEM((SEG, DM), F32),
            pltpu.VMEM((AHEAD, DM), BF16),
            pltpu.VMEM((3, RING, H * DH), F32),
            pltpu.SemaphoreType.DMA((15,)),
        ],
        compiler_params=pltpu.CompilerParams(vmem_limit_bytes=120 * 1024 * 1024),
    )(A_x.reshape(S, DM), A_mem0.reshape(M, DM), A_Wq, A_Wk, A_Wv, A_Wo.reshape(H * DH, DM),
      B_w_r.T, B_w_i.T, *_dft_constants())
    return out.reshape(1, S, DM)
```

```python
import math

import jax
import jax.numpy as jnp
import ml_dtypes
import numpy as np
from jax.experimental import pallas as pl
from jax.experimental.pallas import tpu as pltpu

S, DM, H, DH, M, SEG = 2048, 640, 32, 128, 8, 32
L = M + SEG
NSEG = S // SEG
DF = DM // 2 + 1
G = 4
NG = H // G
AHEAD, RING = 288, 384
UNROLL, CU, KU, NB = 2, 4, 8, 64
WP, FP = 321, 129
F32, BF16, U32 = jnp.float32, jnp.bfloat16, jnp.uint32
C1, C2 = math.cos(2 * math.pi / 5), math.cos(4 * math.pi / 5)
S1, S2 = math.sin(2 * math.pi / 5), math.sin(4 * math.pi / 5)


def _dft_constants():
    bf = ml_dtypes.bfloat16
    d2 = np.arange(128)
    fwd = np.zeros((3, 256, 256))
    inv = np.zeros((3, 256, 256))
    scale = 1.0 / (DM * S)
    for r in range(3):
        for j in range(128 if r else 65):
            sg = -1.0 if r and j >= 64 else 1.0
            k = r + 5 * j if sg > 0 else DM - (5 - r + 5 * (j - 64))
            th = 2 * np.pi * ((d2 * k) % DM) / DM
            c, s = np.cos(th), np.sin(th)
            if k in (0, DM // 2):
                s = np.zeros(128)
            fwd[r, :128, j] = c
            fwd[r, :128, 128 + j] = -sg * s
            if r:
                fwd[r, 128:, j] = -s
                fwd[r, 128:, 128 + j] = -sg * c
            w = scale * (1.0 if k in (0, DM // 2) else 2.0)
            inv[r, j, :128] = w * c
            inv[r, 128 + j, :128] = -w * sg * s
            if r:
                inv[r, j, 128:] = w * s
                inv[r, 128 + j, 128:] = w * sg * c
    sf = np.zeros((16, 256, 256))
    for k1 in range(16):
        m = k1 + 16 * np.arange(128)
        th = 2 * np.pi * ((m[:, None] * d2[None, :]) % S) / S
        fr, fi = np.cos(th), -np.sin(th)
        sf[k1] = np.block([[fr, -fi], [fi, fr]])
    si = np.transpose(sf, (0, 2, 1))
    sf = sf.reshape(16, 256, 2, 128).swapaxes(2, 3).reshape(16, 256, 256)

    def row_pairs(a):
        a = a.reshape(384, 2, 256).astype(bf).view(np.uint16).astype(np.uint32)
        return a[:, 0] | a[:, 1] << 16

    return (row_pairs(fwd), row_pairs(inv),
            sf.astype(bf), np.ascontiguousarray(si).astype(bf))


def _mm(a, b):
    return jnp.dot(a, b, preferred_element_type=F32)


def _layernorm(x):
    m = jnp.sum(x, axis=-1, keepdims=True) * (1.0 / DM)
    xc = x - m
    v = jnp.sum(xc * xc, axis=-1, keepdims=True) * (1.0 / DM)
    return xc * jax.lax.rsqrt(v + 1e-5)


def _tiles(x):
    return [x[:, i * 128:(i + 1) * 128] for i in range(x.shape[1] // 128)]


def _radix5(x):
    x0, x1, x2, x3, x4 = _tiles(x)
    a1, a2, b1, b2 = x1 + x4, x2 + x3, x1 - x4, x2 - x3
    return jnp.concatenate([x0 + a1 + a2,
                            x0 + C1 * a1 + C2 * a2, S1 * b1 + S2 * b2,
                            x0 + C2 * a1 + C1 * a2, S2 * b1 - S1 * b2], axis=1)


def _inv_radix5(t):
    t0, t1r, t1i, t2r, t2i = _tiles(t)
    a1, b1 = t0 + C1 * t1r + C2 * t2r, S1 * t1i + S2 * t2i
    a2, b2 = t0 + C2 * t1r + C1 * t2r, S2 * t1i - S1 * t2i
    return jnp.concatenate([t0 + t1r + t2r, a1 - b1, a2 - b2, a2 + b2, a1 + b1], axis=1)


def _dft4(z, sign):
    (ar, ai), (br, bi), (cr, ci), (dr, di) = z
    pr, pi, mr, mi = ar + cr, ai + ci, ar - cr, ai - ci
    qr, qi, nr, ni = br + dr, bi + di, br - dr, bi - di
    lo, hi = (mr + ni, mi - nr), (mr - ni, mi + nr)
    if sign > 0:
        lo, hi = hi, lo
    return [(pr + qr, pi + qi), lo, (pr - qr, pi - qi), hi]


def _twiddle16(z, e, sign):
    zr, zi = z
    if e == 0:
        return z
    if e == 4:
        return (-zi, zr) if sign > 0 else (zi, -zr)
    c, s = math.cos(math.pi * e / 8), sign * math.sin(math.pi * e / 8)
    if e in (2, 6):
        if c * s > 0:
            return (zr - zi) * c, (zr + zi) * c
        return (zr + zi) * c, (zi - zr) * c
    return zr * c - zi * s, zr * s + zi * c


def _dft16(z, sign):
    u = [_dft4([z[4 * a + b] for a in range(4)], sign) for b in range(4)]
    out = [None] * 16
    for c in range(4):
        v = _dft4([_twiddle16(u[b][c], b * c, sign) for b in range(4)], sign)
        for d in range(4):
            out[c + 4 * d] = v[d]
    return out


def _kernel(x_hbm, mem_ref, wq_hbm, wk_hbm, wv_hbm, wo_hbm, wr_hbm, wi_hbm,
            df_hbm, di_hbm, sf_hbm, si_hbm, out_hbm,
            raw_ref, w_ref, wo_ref, flt_raw, tmp_ref, flt_ref,
            df_ref, di_ref, sf_ref, si_ref,
            x_ref, io_ref, r_ref, z_ref, u_ref, hn_ref, ao_ref, hb_ref, qkv_ref, sems):
    halves = [(i, j) for i in range(3) for j in range(2)]
    head, rest = pl.ds(0, AHEAD), pl.ds(AHEAD, S - AHEAD)
    copies = [pltpu.make_async_copy(src, dst, sems.at[i]) for i, (src, dst) in enumerate(
        [((wq_hbm, wk_hbm, wv_hbm)[i].at[:, pl.ds(16 * j, 16), :], raw_ref.at[2 * i + j]) for i, j in halves]
        + [(x_hbm.at[rest], io_ref.at[rest]), (wo_hbm, wo_ref),
           (wr_hbm, flt_raw.at[0]), (wi_hbm, flt_raw.at[1]),
           (df_hbm, df_ref), (di_hbm, di_ref), (sf_hbm, sf_ref), (si_hbm, si_ref),
           (x_hbm.at[head], io_ref.at[head])])]

    def rows(i, n):
        return pl.ds(pl.multiple_of(i * n, n), n)

    def weights(i, g, k):
        tiles = []
        for hd in range(g * G, (g + 1) * G):
            start = ((2 * i + hd // 16) * 16 + hd % 2 * 8 + hd % 16 // 2) * WP + k * 64
            tiles.append(w_ref[start:start + 64, :])
        return pltpu.bitcast(jnp.concatenate(tiles, axis=1), BF16)

    def project(h, i, g):
        acc = None
        for k in range(DM // 128):
            t = _mm(h[:, k * 128:(k + 1) * 128], weights(i, g, k))
            acc = t if acc is None else acc + t
        return acc

    def load_rows(c):
        x = io_ref[rows(c, SEG), :].astype(F32)
        x_ref[rows(c, SEG), :] = x
        return x

    copies[14].start()
    copies[0].start()
    flt_raw[2, :, :128] = jnp.zeros((DF, 128), BF16)
    ao_ref[...] = jnp.zeros((SEG, DM), F32)
    copies[14].wait()
    copies[1].start()

    @pl.loop(0, AHEAD // SEG)
    def _(c):
        hb_ref[rows(c, SEG), :] = _layernorm(load_rows(c)).astype(BF16)

    for n, (i, j) in enumerate(halves):
        copies[n].wait()
        if n < 3:
            copies[2 * n + 2].start()
            copies[2 * n + 3].start()

        @pl.loop(0, DM // 32)
        def _(c):
            v = pltpu.bitcast(raw_ref[n, rows(c, 32)].reshape(32 * 16, DH), U32)
            for q in range(16):
                e, o = v[16 * q:16 * q + 8], v[16 * q + 8:16 * q + 16]
                at = n * 16 * WP + c * 16 + q
                w_ref[pl.ds(at, 8, stride=WP), :] = (e & 0xFFFF) | (o << 16)
                w_ref[pl.ds(at + 8 * WP, 8, stride=WP), :] = (e >> 16) | (o & np.uint32(0xFFFF0000))

        if n == 5:
            copies[6].wait()

        @pl.loop(0, AHEAD // 96)
        def _(c):
            for g in range(j * NG // 2, (j + 1) * NG // 2):
                qkv_ref[i, rows(c, 96), g * G * DH:(g + 1) * G * DH] = project(hb_ref[rows(c, 96), :], i, g)
            if n == 5:
                per = -(-(NSEG - AHEAD // SEG) // (AHEAD // 96))
                for q in range(per):
                    load_rows(jnp.minimum(AHEAD // SEG + c * per + q, NSEG - 1))

    copies[7].wait()
    for c in copies[8:14]:
        c.start()

    def prepare_filter(p, c):
        blk = pl.ds(pl.multiple_of(c * 128, 128), 128)
        tmp_ref[...] = flt_raw[p, :DF - 1, blk].astype(F32)
        last = jnp.concatenate([flt_raw[p, DF - 1:, blk].astype(F32), jnp.zeros((63, 128), F32)], axis=0)
        part = [tmp_ref[pl.ds(k, 64, stride=5), :] for k in range(5)]
        for r in range(3):
            v = jnp.concatenate([part[r], part[5 - r] if r else last], axis=0).T
            for q in range(16):
                at = ((p % 2 * 3 + r) * 16 + q % 2 * 8) * FP + c * 8 + q // 2
                flt_ref[pl.ds(at, 8, stride=FP), :] = v[8 * q:8 * q + 8]

    def enter(rs):
        hn_ref[...] = _layernorm(x_ref[rs, :])

    def leave(s):
        x = x_ref[rows(s, SEG), :] + ao_ref[...]
        x_ref[rows(s, SEG), :] = x
        r_ref[rows(s, SEG), :] = _radix5(_layernorm(x))

    ri = jax.lax.broadcasted_iota(jnp.int32, (L, L), 0)
    ci = jax.lax.broadcasted_iota(jnp.int32, (L, L), 1)
    mask = (ri < M) | (ri >= ci)

    def segment(s, mem, early):
        h = jnp.concatenate([mem, hn_ref[:SEG - M if early else SEG, :]], axis=0)
        leave(jnp.maximum(s - 1, 0))
        if early:
            enter(pl.ds(pl.multiple_of(AHEAD + (s + 1) * (SEG - M), 8), SEG))
            piece = jnp.clip(s - 4, 0, 31)
            prepare_filter(jnp.where(s < 4, 2, piece // 16), piece % 16)
            put = pl.ds(pl.multiple_of((AHEAD + s * (SEG - M)) % RING, 8), SEG - M)
            get = pl.ds(pl.multiple_of(s * SEG % RING, SEG), SEG)
        else:
            enter(rows(jnp.minimum(s + 1, NSEG - 1), SEG))

        def proj(i, g):
            y = project(h, i, g)
            if early:
                cols = slice(g * G * DH, (g + 1) * G * DH)
                qkv_ref[i, put, cols] = y[M:]
                y = jnp.concatenate([y[:M], qkv_ref[i, get, cols]], axis=0)
            return y

        def scores(q, k):
            res = []
            for qh, kh in zip(_tiles(q), _tiles(k)):
                sc = jax.lax.dot_general(qh, kh.astype(BF16), (((1,), (1,)), ((), ())),
                                         preferred_element_type=F32)
                sc = jnp.where(mask, sc * DH ** -0.5, -1e9)
                e = jnp.exp(sc - jnp.max(sc, axis=-1, keepdims=True))
                d = jnp.sum(e, axis=-1, keepdims=True)
                r = pltpu.reciprocal(d, approx=True)
                res.append((e, r * (2.0 - d * r)))
            return res

        def values(es, v):
            return jnp.concatenate(
                [_mm(e, vh.astype(BF16)) * r for (e, r), vh in zip(es, _tiles(v))], axis=1)

        def project_out(o, g):
            return _mm(o, wo_ref[g * G * DH:(g + 1) * G * DH, :])

        os_, es, v = [], None, None
        for g in range(NG):
            q, k = proj(0, g), proj(1, g)
            if g:
                os_.append(values(es, v))
            v = proj(2, g)
            es = scores(q, k)
        out = project_out(os_[0], 0)
        for g in range(1, NG - 2):
            out = out + project_out(os_[g], g)
        os_.append(values(es, v))
        for g in range(NG - 2, NG):
            out = out + project_out(os_[g], g)
        ao_ref[...] = out[M:]
        return out[:M]

    def segments(first, last, mem, early):
        def body(i, mem):
            if early:
                @pl.when(i == 4 // UNROLL)
                def _():
                    copies[8].wait()
                    copies[9].wait()
            for q in range(UNROLL):
                mem = segment(i * UNROLL + q, mem, early)
            return mem
        return jax.lax.fori_loop(first // UNROLL, last // UNROLL, body, mem)

    def out_copy(c):
        rs = rows(c, 512)
        return pltpu.make_async_copy(io_ref.at[rs], out_hbm.at[rs], sems.at[c])

    def spectral(layer):
        @pl.loop(0, 8 // CU)
        def _(i):
            for q in range(CU):
                groups = [(i * CU + q) * 2 + o for o in range(2)]
                for r in (1, 2, 0):
                    src = slice(r * 256 - 128, r * 256 + 128) if r else slice(0, 128)
                    lhs = jnp.concatenate([r_ref[pl.ds(pl.multiple_of(n1 * 128 + c * 8, 8), 8), src]
                                           for c in groups for n1 in range(16)], axis=0)
                    y = _mm(lhs, pltpu.bitcast(df_ref[r * 128:r * 128 + lhs.shape[1] // 2, :], BF16))
                    for o, c in enumerate(groups):
                        y8 = [y[(16 * o + n1) * 8:(16 * o + n1 + 1) * 8] for n1 in range(16)]
                        for k1, z in enumerate(_dft16([_tiles(v) for v in y8], -1)):
                            z_ref[k1, rows(c, 8), r * 128:(r + 1) * 128] = pltpu.pack_elementwise(
                                list(z), packed_dtype=BF16)

        @pl.loop(0, 16 // KU)
        def _(i):
            ys = []
            for q in range(KU + 2):
                if q < KU:
                    k1 = i * KU + q
                    x = _mm(sf_ref[k1], pltpu.bitcast(z_ref[k1], BF16))
                    wr, wi = (jnp.concatenate([flt_ref[pl.ds(((p * 3 + r) * 16 + k1) * FP, 128), :]
                                               for r in range(3)], axis=1) for p in range(2))
                    xr, xi = x[:128], x[128:]
                    ys.append(jnp.concatenate([xr * wr - xi * wi, xr * wi + xi * wr], axis=0).astype(BF16))
                if q >= 2:
                    qkv_ref[i, :256, (q - 2) * 384:(q - 1) * 384] = _mm(si_ref[i * KU + q - 2], ys[q - 2])

        def ucols(k1, r):
            return slice(k1 % 8 * 384 + r * 128, k1 % 8 * 384 + (r + 1) * 128)

        @pl.loop(0, 16)
        def _(c):
            for r in range(3):
                cols = slice(r * 128, (r + 1) * 128)
                z = _dft16([(qkv_ref[k1 // 8, rows(c, 8), ucols(k1, r)], qkv_ref[k1 // 8, rows(16 + c, 8), ucols(k1, r)])
                            for k1 in range(16)], 1)
                for n1 in range(16):
                    u_ref[n1, rows(c, 8), cols], u_ref[n1, rows(16 + c, 8), cols] = z[n1]

        @pl.loop(0, 4)
        def _(i):
            for q in range(512 // NB):
                n1, n2 = i * 4 + q * NB // 128, q * NB % 128
                t = jnp.concatenate(
                    [_mm(jnp.concatenate([u_ref[n1, p + n2:p + n2 + NB, r * 128:(r + 1) * 128] for p in (0, 128)], axis=1),
                         pltpu.bitcast(di_ref[r * 128:(r + 1) * 128, :256 if r else 128], BF16))
                     for r in range(3)], axis=1)
                rs = rows(i * (512 // NB) + q, NB)
                x = x_ref[rs, :] + _inv_radix5(t)
                x_ref[rs, :] = x
                io_ref[rs, :] = x.astype(BF16)
            pl.when(layer == 1)(lambda: out_copy(i).start())

    mem0 = mem_ref[...].astype(F32)
    enter(pl.ds(AHEAD, SEG))
    mem1 = segments(0, AHEAD // M, mem0, True)
    for c in copies[10:14]:
        c.wait()

    @pl.loop(0, 2)
    def _(layer):
        first = jnp.where(layer == 0, AHEAD // M, 0)
        enter(rows(first, SEG))
        segments(first, NSEG, jnp.where(layer == 0, mem1, mem0), False)
        leave(NSEG - 1)
        ao_ref[...] = jnp.zeros((SEG, DM), F32)
        spectral(layer)

    for i in range(4):
        out_copy(i).wait()


@jax.jit
def pallas_interleave_layers__memory_aug_recurrent_mem_tr__spectral_gfnet__prompt_kernel(
    A_x: jax.Array,
    A_mem0: jax.Array,
    A_Wq: jax.Array,
    A_Wk: jax.Array,
    A_Wv: jax.Array,
    A_Wo: jax.Array,
    A_seg_len: jax.Array,
    B_x: jax.Array,
    B_w_r: jax.Array,
    B_w_i: jax.Array,
):
    del A_seg_len, B_x
    assert A_x.shape == (1, S, DM) and A_mem0.shape == (1, M, DM) and A_Wq.shape == (DM, H, DH)
    hbm = pl.BlockSpec(memory_space=pltpu.HBM)
    out = pl.pallas_call(
        _kernel,
        out_shape=jax.ShapeDtypeStruct((S, DM), BF16),
        in_specs=[hbm, pl.BlockSpec(memory_space=pltpu.VMEM)] + [hbm] * 10,
        out_specs=hbm,
        scratch_shapes=[
            pltpu.VMEM((6, DM, 16, DH), BF16),
            pltpu.VMEM((3 * H * WP, DH), U32),
            pltpu.VMEM((H * DH, DM), BF16),
            pltpu.VMEM((3, DF, S), BF16),
            pltpu.VMEM((DF - 1, 128), F32),
            pltpu.VMEM((6 * 16 * FP, 128), F32),
            pltpu.VMEM((384, 256), U32),
            pltpu.VMEM((384, 256), U32),
            pltpu.VMEM((16, 256, 256), BF16),
            pltpu.VMEM((16, 256, 256), BF16),
            pltpu.VMEM((S, DM), F32),
            pltpu.VMEM((S, DM), BF16),
            pltpu.VMEM((S, DM), F32),
            pltpu.VMEM((16, 128, 384), U32),
            pltpu.VMEM((16, 256, 384), F32),
            pltpu.VMEM((SEG, DM), F32),
            pltpu.VMEM((SEG, DM), F32),
            pltpu.VMEM((AHEAD, DM), BF16),
            pltpu.VMEM((3, RING, H * DH), F32),
            pltpu.SemaphoreType.DMA((15,)),
        ],
        compiler_params=pltpu.CompilerParams(vmem_limit_bytes=120 * 1024 * 1024),
    )(A_x.reshape(S, DM), A_mem0.reshape(M, DM), A_Wq, A_Wk, A_Wv, A_Wo.reshape(H * DH, DM),
      B_w_r.T, B_w_i.T, *_dft_constants())
    return out.reshape(1, S, DM)
```

```python
import math

import jax
import jax.numpy as jnp
import ml_dtypes
import numpy as np
from jax.experimental import pallas as pl
from jax.experimental.pallas import tpu as pltpu

S, DM, H, DH, M, SEG = 2048, 640, 32, 128, 8, 32
L = M + SEG
NSEG = S // SEG
DF = DM // 2 + 1
G = 4
NG = H // G
AHEAD, RING = 288, 384
UNROLL, CU, KU, NB = 2, 4, 8, 64
HEAD = 448
WP, FP = 321, 129
F32, BF16, U32 = jnp.float32, jnp.bfloat16, jnp.uint32
C1, C2 = math.cos(2 * math.pi / 5), math.cos(4 * math.pi / 5)
S1, S2 = math.sin(2 * math.pi / 5), math.sin(4 * math.pi / 5)


def _dft_constants():
    bf = ml_dtypes.bfloat16
    d2 = np.arange(128)
    fwd = np.zeros((3, 256, 256))
    inv = np.zeros((3, 256, 256))
    scale = 1.0 / (DM * S)
    for r in range(3):
        for j in range(128 if r else 65):
            sg = -1.0 if r and j >= 64 else 1.0
            k = r + 5 * j if sg > 0 else DM - (5 - r + 5 * (j - 64))
            th = 2 * np.pi * ((d2 * k) % DM) / DM
            c, s = np.cos(th), np.sin(th)
            if k in (0, DM // 2):
                s = np.zeros(128)
            fwd[r, :128, j] = c
            fwd[r, :128, 128 + j] = -sg * s
            if r:
                fwd[r, 128:, j] = -s
                fwd[r, 128:, 128 + j] = -sg * c
            w = scale * (1.0 if k in (0, DM // 2) else 2.0)
            inv[r, j, :128] = w * c
            inv[r, 128 + j, :128] = -w * sg * s
            if r:
                inv[r, j, 128:] = w * s
                inv[r, 128 + j, 128:] = w * sg * c
    sf = np.zeros((16, 256, 256))
    for k1 in range(16):
        m = k1 + 16 * np.arange(128)
        th = 2 * np.pi * ((m[:, None] * d2[None, :]) % S) / S
        fr, fi = np.cos(th), -np.sin(th)
        sf[k1] = np.block([[fr, -fi], [fi, fr]])
    si = np.transpose(sf, (0, 2, 1))
    sf = sf.reshape(16, 256, 2, 128).swapaxes(2, 3).reshape(16, 256, 256)

    def row_pairs(a):
        a = a.reshape(384, 2, 256).astype(bf).view(np.uint16).astype(np.uint32)
        return a[:, 0] | a[:, 1] << 16

    return (row_pairs(fwd), row_pairs(inv),
            sf.astype(bf), np.ascontiguousarray(si).astype(bf))


def _mm(a, b):
    return jnp.dot(a, b, preferred_element_type=F32)


def _layernorm(x):
    m = jnp.sum(x, axis=-1, keepdims=True) * (1.0 / DM)
    xc = x - m
    v = jnp.sum(xc * xc, axis=-1, keepdims=True) * (1.0 / DM)
    return xc * jax.lax.rsqrt(v + 1e-5)


def _tiles(x):
    return [x[:, i * 128:(i + 1) * 128] for i in range(x.shape[1] // 128)]


def _radix5(x):
    x0, x1, x2, x3, x4 = _tiles(x)
    a1, a2, b1, b2 = x1 + x4, x2 + x3, x1 - x4, x2 - x3
    return jnp.concatenate([x0 + a1 + a2,
                            x0 + C1 * a1 + C2 * a2, S1 * b1 + S2 * b2,
                            x0 + C2 * a1 + C1 * a2, S2 * b1 - S1 * b2], axis=1)


def _inv_radix5(t):
    t0, t1r, t1i, t2r, t2i = _tiles(t)
    a1, b1 = t0 + C1 * t1r + C2 * t2r, S1 * t1i + S2 * t2i
    a2, b2 = t0 + C2 * t1r + C1 * t2r, S2 * t1i - S1 * t2i
    return jnp.concatenate([t0 + t1r + t2r, a1 - b1, a2 - b2, a2 + b2, a1 + b1], axis=1)


def _dft4(z, sign):
    (ar, ai), (br, bi), (cr, ci), (dr, di) = z
    pr, pi, mr, mi = ar + cr, ai + ci, ar - cr, ai - ci
    qr, qi, nr, ni = br + dr, bi + di, br - dr, bi - di
    lo, hi = (mr + ni, mi - nr), (mr - ni, mi + nr)
    if sign > 0:
        lo, hi = hi, lo
    return [(pr + qr, pi + qi), lo, (pr - qr, pi - qi), hi]


def _twiddle16(z, e, sign):
    zr, zi = z
    if e == 0:
        return z
    if e == 4:
        return (-zi, zr) if sign > 0 else (zi, -zr)
    c, s = math.cos(math.pi * e / 8), sign * math.sin(math.pi * e / 8)
    if e in (2, 6):
        if c * s > 0:
            return (zr - zi) * c, (zr + zi) * c
        return (zr + zi) * c, (zi - zr) * c
    return zr * c - zi * s, zr * s + zi * c


def _dft16(z, sign):
    u = [_dft4([z[4 * a + b] for a in range(4)], sign) for b in range(4)]
    out = [None] * 16
    for c in range(4):
        v = _dft4([_twiddle16(u[b][c], b * c, sign) for b in range(4)], sign)
        for d in range(4):
            out[c + 4 * d] = v[d]
    return out


def _kernel(x_hbm, mem_ref, wq_hbm, wk_hbm, wv_hbm, wo_hbm, wr_hbm, wi_hbm,
            df_hbm, di_hbm, sf_hbm, si_hbm, out_hbm,
            raw_ref, w_ref, wo_ref, flt_raw, tmp_ref, flt_ref,
            df_ref, di_ref, sf_ref, si_ref,
            x_ref, io_ref, r_ref, z_ref, u_ref, hn_ref, ao_ref, hb_ref, qkv_ref, sems):
    head, rest = pl.ds(0, HEAD), pl.ds(HEAD, S - HEAD)
    copies = [pltpu.make_async_copy(src, dst, sems.at[i]) for i, (src, dst) in enumerate(
        [(w.at[:, pl.ds(16 * j, 16), :], raw_ref.at[2 * i + j])
         for i, w in enumerate((wq_hbm, wk_hbm, wv_hbm)) for j in range(2)]
        + [(wo_hbm, wo_ref), (x_hbm.at[rest], io_ref.at[rest]),
           (wr_hbm, flt_raw.at[0]), (wi_hbm, flt_raw.at[1]),
           (df_hbm, df_ref), (di_hbm, di_ref), (sf_hbm, sf_ref), (si_hbm, si_ref),
           (x_hbm.at[head], io_ref.at[head])])]

    def rows(i, n):
        return pl.ds(pl.multiple_of(i * n, n), n)

    def weights(i, g, k):
        tiles = [w_ref[pl.ds((i * 32 + hd // 16 * 16 + hd % 2 * 8 + hd % 16 // 2) * WP + k * 64, 64), :]
                 for hd in range(g * G, (g + 1) * G)]
        return pltpu.bitcast(jnp.concatenate(tiles, axis=1), BF16)

    def project(h, i, g, between=None):
        acc = None
        for k in range(DM // 128):
            t = _mm(h[:, k * 128:(k + 1) * 128], weights(i, g, k))
            acc = t if acc is None else acc + t
            if between:
                between(g % 4 * 5 + k)
        return acc

    def load_rows(rs):
        x = io_ref[rs, :].astype(F32)
        x_ref[rs, :] = x
        return x

    def repack(i, j, c):
        v = pltpu.bitcast(raw_ref[2 * i + j, rows(c, 32)].reshape(32 * 16, DH), U32)
        for q in range(16):
            e, o = v[16 * q:16 * q + 8], v[16 * q + 8:16 * q + 16]
            at = (2 * i + j) * 16 * WP + c * 16 + q
            w_ref[pl.ds(at, 8, stride=WP), :] = (e & 0xFFFF) | (o << 16)
            w_ref[pl.ds(at + 8 * WP, 8, stride=WP), :] = (e >> 16) | (o & np.uint32(0xFFFF0000))

    copies[14].start()
    copies[0].start()
    flt_raw[2, :, :128] = jnp.zeros((DF, 128), BF16)
    ao_ref[...] = jnp.zeros((SEG, DM), F32)
    copies[14].wait()

    @pl.loop(0, AHEAD // 48)
    def _(c):
        hb_ref[rows(c, 48), :] = _layernorm(load_rows(rows(c, 48))).astype(BF16)

    load_rows(pl.ds(AHEAD, HEAD - AHEAD))
    copies[1].start()
    copies[0].wait()
    pl.loop(0, DM // 32)(lambda c: repack(0, 0, c))

    @pl.loop(0, 3)
    def _(i):
        for j in range(2):
            def project_ahead(c, between=None):
                for g in range(j * NG // 2, (j + 1) * NG // 2):
                    qkv_ref[i, rows(c, 96), g * G * DH:(g + 1) * G * DH] = project(
                        hb_ref[rows(c, 96), :], i, g, between)

            for n in range(j, 5, 2):
                pl.when(i == n // 2)(copies[n + 2].start)
            pl.loop(0, AHEAD // 96 - 1)(project_ahead)
            for n in range(j, 5, 2):
                pl.when(i == n // 2)(copies[n + 1].wait)
            project_ahead(AHEAD // 96 - 1, lambda c: repack(jnp.minimum(i + j, 2), 1 - j, c))

    copies[6].wait()
    for c in copies[7:14]:
        c.start()

    def prepare_filter(p, c):
        blk = pl.ds(pl.multiple_of(c * 128, 128), 128)
        tmp_ref[...] = flt_raw[p, :DF - 1, blk].astype(F32)
        last = jnp.concatenate([flt_raw[p, DF - 1:, blk].astype(F32), jnp.zeros((63, 128), F32)], axis=0)
        part = [tmp_ref[pl.ds(k, 64, stride=5), :] for k in range(5)]
        for r in range(3):
            v = jnp.concatenate([part[r], part[5 - r] if r else last], axis=0).T
            for q in range(16):
                at = ((p % 2 * 3 + r) * 16 + q % 2 * 8) * FP + c * 8 + q // 2
                flt_ref[pl.ds(at, 8, stride=FP), :] = v[8 * q:8 * q + 8]

    def enter(rs):
        hn_ref[...] = _layernorm(x_ref[rs, :])

    def leave(s):
        x = x_ref[rows(s, SEG), :] + ao_ref[...]
        x_ref[rows(s, SEG), :] = x
        r_ref[rows(s, SEG), :] = _radix5(_layernorm(x))

    ri = jax.lax.broadcasted_iota(jnp.int32, (L, L), 0)
    ci = jax.lax.broadcasted_iota(jnp.int32, (L, L), 1)
    mask = (ri < M) | (ri >= ci)

    def segment(s, mem, early):
        h = jnp.concatenate([mem, hn_ref[:SEG - M if early else SEG, :]], axis=0)
        leave(jnp.maximum(s - 1, 0))
        if early:
            enter(pl.ds(pl.multiple_of(AHEAD + (s + 1) * (SEG - M), 8), SEG))
            load_rows(rows(jnp.clip(HEAD // 64 + s - 4, HEAD // 64 - 1, S // 64 - 1), 64))
            piece = jnp.clip(s - 4, 0, 31)
            prepare_filter(jnp.where(s < 4, 2, piece // 16), piece % 16)
            put = pl.ds(pl.multiple_of((AHEAD + s * (SEG - M)) % RING, 8), SEG - M)
            get = pl.ds(pl.multiple_of(s * SEG % RING, SEG), SEG)
        else:
            enter(rows(jnp.minimum(s + 1, NSEG - 1), SEG))

        def proj(i, g):
            y = project(h, i, g)
            if early:
                cols = slice(g * G * DH, (g + 1) * G * DH)
                qkv_ref[i, put, cols] = y[M:]
                y = jnp.concatenate([y[:M], qkv_ref[i, get, cols]], axis=0)
            return y

        def scores(q, k):
            res = []
            for qh, kh in zip(_tiles(q), _tiles(k)):
                sc = jax.lax.dot_general(qh, kh.astype(BF16), (((1,), (1,)), ((), ())),
                                         preferred_element_type=F32)
                sc = jnp.where(mask, sc * DH ** -0.5, -1e9)
                e = jnp.exp(sc - jnp.max(sc, axis=-1, keepdims=True))
                d = jnp.sum(e, axis=-1, keepdims=True)
                r = pltpu.reciprocal(d, approx=True)
                res.append((e, r * (2.0 - d * r)))
            return res

        def values(es, v):
            return jnp.concatenate(
                [_mm(e, vh.astype(BF16)) * r for (e, r), vh in zip(es, _tiles(v))], axis=1)

        def project_out(o, g):
            return _mm(o, wo_ref[g * G * DH:(g + 1) * G * DH, :])

        os_, es, v = [], None, None
        for g in range(NG):
            q, k = proj(0, g), proj(1, g)
            if g:
                os_.append(values(es, v))
            v = proj(2, g)
            es = scores(q, k)
        out = project_out(os_[0], 0)
        for g in range(1, NG - 2):
            out = out + project_out(os_[g], g)
        os_.append(values(es, v))
        for g in range(NG - 2, NG):
            out = out + project_out(os_[g], g)
        ao_ref[...] = out[M:]
        return out[:M]

    def segments(first, last, mem, early):
        def body(i, mem):
            if early:
                @pl.when(i == 4 // UNROLL)
                def _():
                    for c in copies[7:10]:
                        c.wait()
            for q in range(UNROLL):
                mem = segment(i * UNROLL + q, mem, early)
            return mem
        return jax.lax.fori_loop(first // UNROLL, last // UNROLL, body, mem)

    def out_copy(c):
        rs = rows(c, 512)
        return pltpu.make_async_copy(io_ref.at[rs], out_hbm.at[rs], sems.at[c])

    def spectral(layer):
        @pl.loop(0, 8 // CU)
        def _(i):
            for q in range(CU):
                groups = [(i * CU + q) * 2 + o for o in range(2)]
                for r in (1, 2, 0):
                    src = slice(r * 256 - 128, r * 256 + 128) if r else slice(0, 128)
                    lhs = jnp.concatenate([r_ref[pl.ds(pl.multiple_of(n1 * 128 + c * 8, 8), 8), src]
                                           for c in groups for n1 in range(16)], axis=0)
                    y = _mm(lhs, pltpu.bitcast(df_ref[r * 128:r * 128 + lhs.shape[1] // 2, :], BF16))
                    for o, c in enumerate(groups):
                        y8 = [y[(16 * o + n1) * 8:(16 * o + n1 + 1) * 8] for n1 in range(16)]
                        for k1, z in enumerate(_dft16([_tiles(v) for v in y8], -1)):
                            z_ref[k1, rows(c, 8), r * 128:(r + 1) * 128] = pltpu.pack_elementwise(
                                list(z), packed_dtype=BF16)

        @pl.loop(0, 16 // KU)
        def _(i):
            ys = []
            for q in range(KU + 2):
                if q < KU:
                    k1 = i * KU + q
                    x = _mm(sf_ref[k1], pltpu.bitcast(z_ref[k1], BF16))
                    wr, wi = (jnp.concatenate([flt_ref[pl.ds(((p * 3 + r) * 16 + k1) * FP, 128), :]
                                               for r in range(3)], axis=1) for p in range(2))
                    xr, xi = x[:128], x[128:]
                    ys.append(jnp.concatenate([xr * wr - xi * wi, xr * wi + xi * wr], axis=0).astype(BF16))
                if q >= 2:
                    qkv_ref[i, :256, (q - 2) * 384:(q - 1) * 384] = _mm(si_ref[i * KU + q - 2], ys[q - 2])

        def ucols(k1, r):
            return slice(k1 % 8 * 384 + r * 128, k1 % 8 * 384 + (r + 1) * 128)

        @pl.loop(0, 16)
        def _(c):
            for r in range(3):
                cols = slice(r * 128, (r + 1) * 128)
                z = _dft16([(qkv_ref[k1 // 8, rows(c, 8), ucols(k1, r)], qkv_ref[k1 // 8, rows(16 + c, 8), ucols(k1, r)])
                            for k1 in range(16)], 1)
                for n1 in range(16):
                    u_ref[n1, rows(c, 8), cols], u_ref[n1, rows(16 + c, 8), cols] = z[n1]

        @pl.loop(0, 4)
        def _(i):
            for q in range(512 // NB):
                n1, n2 = i * 4 + q * NB // 128, q * NB % 128
                t = jnp.concatenate(
                    [_mm(jnp.concatenate([u_ref[n1, p + n2:p + n2 + NB, r * 128:(r + 1) * 128] for p in (0, 128)], axis=1),
                         pltpu.bitcast(di_ref[r * 128:(r + 1) * 128, :256 if r else 128], BF16))
                     for r in range(3)], axis=1)
                rs = rows(i * (512 // NB) + q, NB)
                x = x_ref[rs, :] + _inv_radix5(t)
                x_ref[rs, :] = x
                io_ref[rs, :] = x.astype(BF16)
            pl.when(layer == 1)(lambda: out_copy(i).start())

    mem0 = mem_ref[...].astype(F32)
    enter(pl.ds(AHEAD, SEG))
    mem1 = segments(0, AHEAD // M, mem0, True)
    for c in copies[10:14]:
        c.wait()

    @pl.loop(0, 2)
    def _(layer):
        first = jnp.where(layer == 0, AHEAD // M, 0)
        enter(rows(first, SEG))
        segments(first, NSEG, jnp.where(layer == 0, mem1, mem0), False)
        leave(NSEG - 1)
        ao_ref[...] = jnp.zeros((SEG, DM), F32)
        spectral(layer)

    for i in range(4):
        out_copy(i).wait()


@jax.jit
def pallas_interleave_layers__memory_aug_recurrent_mem_tr__spectral_gfnet__prompt_kernel(
    A_x: jax.Array,
    A_mem0: jax.Array,
    A_Wq: jax.Array,
    A_Wk: jax.Array,
    A_Wv: jax.Array,
    A_Wo: jax.Array,
    A_seg_len: jax.Array,
    B_x: jax.Array,
    B_w_r: jax.Array,
    B_w_i: jax.Array,
):
    del A_seg_len, B_x
    assert A_x.shape == (1, S, DM) and A_mem0.shape == (1, M, DM) and A_Wq.shape == (DM, H, DH)
    hbm = pl.BlockSpec(memory_space=pltpu.HBM)
    out = pl.pallas_call(
        _kernel,
        out_shape=jax.ShapeDtypeStruct((S, DM), BF16),
        in_specs=[hbm, pl.BlockSpec(memory_space=pltpu.VMEM)] + [hbm] * 10,
        out_specs=hbm,
        scratch_shapes=[
            pltpu.VMEM((6, DM, 16, DH), BF16),
            pltpu.VMEM((3 * H * WP, DH), U32),
            pltpu.VMEM((H * DH, DM), BF16),
            pltpu.VMEM((3, DF, S), BF16),
            pltpu.VMEM((DF - 1, 128), F32),
            pltpu.VMEM((6 * 16 * FP, 128), F32),
            pltpu.VMEM((384, 256), U32),
            pltpu.VMEM((384, 256), U32),
            pltpu.VMEM((16, 256, 256), BF16),
            pltpu.VMEM((16, 256, 256), BF16),
            pltpu.VMEM((S, DM), F32),
            pltpu.VMEM((S, DM), BF16),
            pltpu.VMEM((S, DM), F32),
            pltpu.VMEM((16, 128, 384), U32),
            pltpu.VMEM((16, 256, 384), F32),
            pltpu.VMEM((SEG, DM), F32),
            pltpu.VMEM((SEG, DM), F32),
            pltpu.VMEM((AHEAD, DM), BF16),
            pltpu.VMEM((3, RING, H * DH), F32),
            pltpu.SemaphoreType.DMA((15,)),
        ],
        compiler_params=pltpu.CompilerParams(vmem_limit_bytes=120 * 1024 * 1024),
    )(A_x.reshape(S, DM), A_mem0.reshape(M, DM), A_Wq, A_Wk, A_Wv, A_Wo.reshape(H * DH, DM),
      B_w_r.T, B_w_i.T, *_dft_constants())
    return out.reshape(1, S, DM)
```

```python
import math

import jax
import jax.numpy as jnp
import ml_dtypes
import numpy as np
from jax.experimental import pallas as pl
from jax.experimental.pallas import tpu as pltpu

S, DM, H, DH, M, SEG = 2048, 640, 32, 128, 8, 32
L = M + SEG
NSEG = S // SEG
DF = DM // 2 + 1
G = 4
NG = H // G
AHEAD, RING = 288, 384
UNROLL, CU = 4, 8
HEAD = 448
UE = 2
WP, FP = 321, 129
F32, BF16, U32 = jnp.float32, jnp.bfloat16, jnp.uint32
C1, C2 = math.cos(2 * math.pi / 5), math.cos(4 * math.pi / 5)
S1, S2 = math.sin(2 * math.pi / 5), math.sin(4 * math.pi / 5)


def _dft_constants():
    def mul3(f):
        return [f.real, f.real + f.imag, f.imag - f.real]

    def unit(n, period):
        return np.exp(2j * np.pi * (n % period) / period)

    def row_pairs(mats):
        a = np.stack(mats).reshape(-1, 64, 2, 128).astype(ml_dtypes.bfloat16).view(np.uint16).astype(np.uint32)
        return a[:, :, 0] | a[:, :, 1] << 16

    n2 = np.arange(128)
    scale = 2.0 / (DM * S)
    k = 5 * n2
    f = unit(n2[:, None] * k, DM) * (k <= DM // 2)
    edge = k % (DM // 2) == 0
    f = np.where(edge, f.real, f)
    w = np.where(edge, 0.5, 1.0)[:, None] * scale
    fwd, inv = [f.real, -f.imag], [w * f.T.real, -w * f.T.imag]
    for r in (1, 2):
        k = np.where(n2 < 64, r + 5 * n2, DM - (5 - r + 5 * (n2 - 64)))
        f = unit(n2[:, None] * k, DM)
        fwd += mul3(f)
        inv += mul3(scale * f.T)
    sf, si = [], []
    for k1 in range(16):
        f = unit((k1 + 16 * n2)[:, None] * n2, S)
        sf += mul3(f.conj())
        si += mul3(f.T)
    return row_pairs(fwd), row_pairs(inv), row_pairs(sf), row_pairs(si)


def _mm(a, b):
    return jnp.dot(a, b, preferred_element_type=F32)


def _layernorm(x):
    m = jnp.sum(x, axis=-1, keepdims=True) * (1.0 / DM)
    xc = x - m
    v = jnp.sum(xc * xc, axis=-1, keepdims=True) * (1.0 / DM)
    return xc * jax.lax.rsqrt(v + 1e-5)


def _tiles(x):
    return [x[:, i * 128:(i + 1) * 128] for i in range(x.shape[1] // 128)]


def _radix5(x):
    x0, x1, x2, x3, x4 = _tiles(x)
    a1, a2, b1, b2 = x1 + x4, x2 + x3, x1 - x4, x2 - x3
    return jnp.concatenate([x0 + a1 + a2,
                            x0 + C1 * a1 + C2 * a2, S1 * b1 + S2 * b2,
                            x0 + C2 * a1 + C1 * a2, S2 * b1 - S1 * b2], axis=1)


def _inv_radix5(t0, t1r, t1i, t2r, t2i):
    a1, b1 = t0 + C1 * t1r + C2 * t2r, S1 * t1i + S2 * t2i
    a2, b2 = t0 + C2 * t1r + C1 * t2r, S2 * t1i - S1 * t2i
    return jnp.concatenate([t0 + t1r + t2r, a1 - b1, a2 - b2, a2 + b2, a1 + b1], axis=1)


def _dft4(z, sign):
    (ar, ai), (br, bi), (cr, ci), (dr, di) = z
    pr, pi, mr, mi = ar + cr, ai + ci, ar - cr, ai - ci
    qr, qi, nr, ni = br + dr, bi + di, br - dr, bi - di
    lo, hi = (mr + ni, mi - nr), (mr - ni, mi + nr)
    if sign > 0:
        lo, hi = hi, lo
    return [(pr + qr, pi + qi), lo, (pr - qr, pi - qi), hi]


def _twiddle16(z, e, sign):
    zr, zi = z
    if e == 0:
        return z
    if e == 4:
        return (-zi, zr) if sign > 0 else (zi, -zr)
    c, s = math.cos(math.pi * e / 8), sign * math.sin(math.pi * e / 8)
    if e in (2, 6):
        if c * s > 0:
            return (zr - zi) * c, (zr + zi) * c
        return (zr + zi) * c, (zi - zr) * c
    return zr * c - zi * s, zr * s + zi * c


def _dft16(z, sign):
    u = [_dft4([z[4 * a + b] for a in range(4)], sign) for b in range(4)]
    out = [None] * 16
    for c in range(4):
        v = _dft4([_twiddle16(u[b][c], b * c, sign) for b in range(4)], sign)
        for d in range(4):
            out[c + 4 * d] = v[d]
    return out


def _kernel(x_hbm, mem_ref, wq_hbm, wk_hbm, wv_hbm, wo_hbm, wr_hbm, wi_hbm,
            df_hbm, di_hbm, sf_hbm, si_hbm, out_hbm,
            raw_ref, w_ref, wo_ref, flt_raw, tmp_ref, flt_ref,
            df_ref, di_ref, sf_ref, si_ref,
            x_ref, io_ref, r_ref, u_ref, hn_ref, ao_ref, hb_ref, qkv_ref, sems):
    head, rest = pl.ds(0, HEAD), pl.ds(HEAD, S - HEAD)
    copies = [pltpu.make_async_copy(src, dst, sems.at[i]) for i, (src, dst) in enumerate(
        [(w.at[:, pl.ds(16 * j, 16), :], raw_ref.at[2 * i + j])
         for i, w in enumerate((wq_hbm, wk_hbm, wv_hbm)) for j in range(2)]
        + [(wo_hbm, wo_ref), (x_hbm.at[rest], io_ref.at[rest]),
           (wr_hbm, flt_raw.at[0]), (wi_hbm, flt_raw.at[1]),
           (df_hbm, df_ref), (di_hbm, di_ref), (sf_hbm, sf_ref), (si_hbm, si_ref),
           (x_hbm.at[head], io_ref.at[head])])]

    def rows(i, n):
        return pl.ds(pl.multiple_of(i * n, n), n)

    def weights(i, g, k):
        tiles = [w_ref[pl.ds((i * 32 + hd // 16 * 16 + hd % 2 * 8 + hd % 16 // 2) * WP + k * 64, 64), :]
                 for hd in range(g * G, (g + 1) * G)]
        return pltpu.bitcast(jnp.concatenate(tiles, axis=1), BF16)

    def project(h, i, g, between=None):
        acc = None
        for k in range(DM // 128):
            t = _mm(h[:, k * 128:(k + 1) * 128], weights(i, g, k))
            acc = t if acc is None else acc + t
            if between:
                between(g % 4 * 5 + k)
        return acc

    def load_rows(rs):
        x = io_ref[rs, :].astype(F32)
        x_ref[rs, :] = x
        return x

    def repack(i, j, c):
        v = pltpu.bitcast(raw_ref[2 * i + j, rows(c, 32)].reshape(32 * 16, DH), U32)
        for q in range(16):
            e, o = v[16 * q:16 * q + 8], v[16 * q + 8:16 * q + 16]
            at = (2 * i + j) * 16 * WP + c * 16 + q
            w_ref[pl.ds(at, 8, stride=WP), :] = (e & 0xFFFF) | (o << 16)
            w_ref[pl.ds(at + 8 * WP, 8, stride=WP), :] = (e >> 16) | (o & np.uint32(0xFFFF0000))

    copies[14].start()
    copies[0].start()
    flt_raw[2, :, :128] = jnp.zeros((DF, 128), BF16)
    ao_ref[...] = jnp.zeros((SEG, DM), F32)
    copies[14].wait()

    @pl.loop(0, AHEAD // 48)
    def _(c):
        hb_ref[rows(c, 48), :] = _layernorm(load_rows(rows(c, 48))).astype(BF16)

    load_rows(pl.ds(AHEAD, HEAD - AHEAD))
    copies[1].start()
    copies[0].wait()
    pl.loop(0, DM // 32)(lambda c: repack(0, 0, c))

    @pl.loop(0, 3)
    def _(i):
        for j in range(2):
            def project_ahead(rs, between=None):
                for g in range(j * NG // 2, (j + 1) * NG // 2):
                    qkv_ref[i, rs, g * G * DH:(g + 1) * G * DH] = project(
                        hb_ref[rs, :], i, g, between)

            for n in range(j, 5, 2):
                pl.when(i == n // 2)(copies[n + 2].start)
            for c in range(AHEAD // 96 - 1):
                project_ahead(pl.ds(c * 96, 96))
            for n in range(j, 5, 2):
                pl.when(i == n // 2)(copies[n + 1].wait)
            project_ahead(pl.ds(AHEAD - 96, 96), lambda c: repack(jnp.minimum(i + j, 2), 1 - j, c))

    copies[6].wait()
    for c in copies[7:14]:
        c.start()

    def prepare_filter(p, c):
        blk = pl.ds(pl.multiple_of(c * 128, 128), 128)
        tmp_ref[:DF - 1, :] = flt_raw[p, :DF - 1, blk].astype(F32)
        last = jnp.concatenate([flt_raw[p, DF - 1:, blk].astype(F32), jnp.zeros((63, 128), F32)], axis=0)
        part = [tmp_ref[pl.ds(k, 64, stride=5), :] for k in range(5)]
        for r in range(3):
            v = jnp.concatenate([part[r], part[5 - r] if r else last], axis=0).T
            for q in range(16):
                at = ((p % 2 * 3 + r) * 16 + q % 2 * 8) * FP + c * 8 + q // 2
                flt_ref[pl.ds(at, 8, stride=FP), :] = v[8 * q:8 * q + 8]

    def enter(rs):
        hn_ref[...] = _layernorm(x_ref[rs, :])

    def leave(s):
        x = x_ref[rows(s, SEG), :] + ao_ref[...]
        x_ref[rows(s, SEG), :] = x
        r_ref[rows(s, SEG), :] = _radix5(_layernorm(x))

    ri = jax.lax.broadcasted_iota(jnp.int32, (L, L), 0)
    ci = jax.lax.broadcasted_iota(jnp.int32, (L, L), 1)
    mask = (ri < M) | (ri >= ci)

    def segment(s, mem, early):
        h = jnp.concatenate([mem, hn_ref[:SEG - M if early else SEG, :]], axis=0)
        leave(jnp.maximum(s - 1, 0))
        if early:
            enter(pl.ds(pl.multiple_of(AHEAD + (s + 1) * (SEG - M), 8), SEG))
            load_rows(rows(jnp.clip(HEAD // 64 + s - 4, HEAD // 64 - 1, S // 64 - 1), 64))
            piece = jnp.clip(s - 4, 0, 31)
            prepare_filter(jnp.where(s < 4, 2, piece // 16), piece % 16)
            put = pl.ds(pl.multiple_of((AHEAD + s * (SEG - M)) % RING, 8), SEG - M)
            get = pl.ds(pl.multiple_of(s * SEG % RING, SEG), SEG)
        else:
            enter(rows(jnp.minimum(s + 1, NSEG - 1), SEG))

        def proj(i, g):
            y = project(h.astype(BF16) if early else h, i, g)
            if early:
                cols = slice(g * G * DH, (g + 1) * G * DH)
                qkv_ref[i, put, cols] = y[M:]
                y = jnp.concatenate([y[:M], qkv_ref[i, get, cols]], axis=0)
            return y

        def scores(q, k):
            res = []
            for qh, kh in zip(_tiles(q), _tiles(k)):
                sc = jax.lax.dot_general(qh, kh.astype(BF16), (((1,), (1,)), ((), ())),
                                         preferred_element_type=F32)
                sc = jnp.where(mask, sc * DH ** -0.5, -1e9)
                e = jnp.exp(sc - jnp.max(sc, axis=-1, keepdims=True))
                d = jnp.sum(e, axis=-1, keepdims=True)
                r = pltpu.reciprocal(d, approx=True)
                res.append((e, r * (2.0 - d * r)))
            return res

        def values(es, v):
            return jnp.concatenate(
                [_mm(e, vh.astype(BF16)) * r for (e, r), vh in zip(es, _tiles(v))], axis=1)

        def project_out(out, g):
            t = _mm(os_[g], wo_ref[g * G * DH:(g + 1) * G * DH, :])
            return t if out is None else out + t

        lag = NG if early else 4
        os_, es, v, out = [], None, None, None
        for g in range(NG):
            q, k = proj(0, g), proj(1, g)
            if g:
                os_.append(values(es, v))
            v = proj(2, g)
            es = scores(q, k)
            if g >= lag:
                out = project_out(out, g - lag)
        for g in range(NG - lag, NG - 2):
            out = project_out(out, g)
        os_.append(values(es, v))
        for g in range(NG - 2, NG):
            out = project_out(out, g)
        ao_ref[...] = out[M:]
        return out[:M]

    def segments(first, last, mem, early):
        unroll = UE if early else UNROLL

        def body(i, mem):
            if early:
                @pl.when(i == 4 // unroll)
                def _():
                    for c in copies[7:10]:
                        c.wait()
            for q in range(unroll):
                mem = segment(i * unroll + q, mem, early)
            return mem
        return jax.lax.fori_loop(first // unroll, last // unroll, body, mem)

    def out_copy(c):
        rs = rows(c, 512)
        return pltpu.make_async_copy(io_ref.at[rs], out_hbm.at[rs], sems.at[c])

    def factor(ref, i):
        return pltpu.bitcast(ref[i], BF16)

    def times(zr, zi, ref, i):
        k = _mm(zr + zi, factor(ref, i))
        return k - _mm(zi, factor(ref, i + 1)), k + _mm(zr, factor(ref, i + 2))

    def applied(ref, i, zr, zi):
        k = _mm(factor(ref, i), (zr + zi).astype(BF16))
        return k - _mm(factor(ref, i + 1), zi.astype(BF16)), k + _mm(factor(ref, i + 2), zr.astype(BF16))

    def spectral(layer):
        sign = jnp.where(jax.lax.broadcasted_iota(jnp.int32, (1, 128), 1) < 64, 1.0, -1.0)

        @pl.loop(0, 16 // CU)
        def _(i):
            for q in range(CU):
                c = i * CU + q
                t0, t1r, t1i, t2r, t2i = _tiles(jnp.concatenate(
                    [r_ref[rows(n1 * 16 + c, 8), :] for n1 in range(16)], axis=0))
                y1, y2 = times(t1r, t1i, df_ref, 2), times(t2r, t2i, df_ref, 5)
                y0 = _mm(t0, factor(df_ref, 0)), _mm(t0, factor(df_ref, 1))
                for r, (yr, yi) in ((1, y1), (2, y2), (0, y0)):
                    yi = yi * -sign if r else yi
                    z = _dft16([(yr[n1 * 8:(n1 + 1) * 8], yi[n1 * 8:(n1 + 1) * 8]) for n1 in range(16)], -1)
                    for k1 in range(16):
                        for p in range(2):
                            u_ref[k1, rows(16 * p + c, 8), r * 128:(r + 1) * 128] = z[k1][p]

        @pl.loop(0, 2)
        def _(i):
            ys = []
            for q in range(8 + 2):
                if q < 8:
                    k1 = i * 8 + q
                    xr, xi = applied(sf_ref, 3 * k1, u_ref[k1, :128], u_ref[k1, 128:])
                    wr, wi = (jnp.concatenate([flt_ref[pl.ds(((p * 3 + r) * 16 + k1) * FP, 128), :]
                                               for r in range(3)], axis=1) for p in range(2))
                    ys.append((xr * wr - xi * wi, xr * wi + xi * wr))
                if q >= 2:
                    qkv_ref[i, :256, (q - 2) * 384:(q - 1) * 384] = jnp.concatenate(
                        applied(si_ref, 3 * (i * 8 + q - 2), *ys[q - 2]), axis=0)

        @pl.loop(0, 16)
        def _(c):
            for r in range(3):
                z = _dft16([[qkv_ref[k1 // 8, rows(16 * p + c, 8), pl.ds(k1 % 8 * 384 + r * 128, 128)]
                             for p in range(2)] for k1 in range(16)], 1)
                for n1 in range(16):
                    for p in range(2):
                        u_ref[n1, rows(16 * p + c, 8), r * 128:(r + 1) * 128] = z[n1][p]

        @pl.loop(0, 4)
        def _(i):
            for q in range(8):
                zr, zi = (_tiles(u_ref[i * 4 + q // 2, pl.ds(128 * p + q % 2 * 64, 64), :]) for p in range(2))
                t0 = _mm(zr[0], factor(di_ref, 0)) + _mm(zi[0], factor(di_ref, 1))
                rs = rows(i * 8 + q, 64)
                x = x_ref[rs, :] + _inv_radix5(t0, *times(zr[1], zi[1] * sign, di_ref, 2),
                                               *times(zr[2], zi[2] * sign, di_ref, 5))
                x_ref[rs, :] = x
                io_ref[rs, :] = x.astype(BF16)
            pl.when(layer == 1)(lambda: out_copy(i).start())

    mem0 = mem_ref[...].astype(F32)
    enter(pl.ds(AHEAD, SEG))
    mem1 = segments(0, AHEAD // M, mem0, True)
    for c in copies[10:14]:
        c.wait()

    @pl.loop(0, 2)
    def _(layer):
        first = jnp.where(layer == 0, AHEAD // M, 0)
        enter(rows(first, SEG))
        segments(first, NSEG, jnp.where(layer == 0, mem1, mem0), False)
        leave(NSEG - 1)
        ao_ref[...] = jnp.zeros((SEG, DM), F32)
        spectral(layer)

    for i in range(4):
        out_copy(i).wait()


@jax.jit
def pallas_interleave_layers__memory_aug_recurrent_mem_tr__spectral_gfnet__prompt_kernel(
    A_x: jax.Array,
    A_mem0: jax.Array,
    A_Wq: jax.Array,
    A_Wk: jax.Array,
    A_Wv: jax.Array,
    A_Wo: jax.Array,
    A_seg_len: jax.Array,
    B_x: jax.Array,
    B_w_r: jax.Array,
    B_w_i: jax.Array,
):
    del A_seg_len, B_x
    assert A_x.shape == (1, S, DM) and A_mem0.shape == (1, M, DM) and A_Wq.shape == (DM, H, DH)
    hbm = pl.BlockSpec(memory_space=pltpu.HBM)
    out = pl.pallas_call(
        _kernel,
        out_shape=jax.ShapeDtypeStruct((S, DM), BF16),
        in_specs=[hbm, pl.BlockSpec(memory_space=pltpu.VMEM)] + [hbm] * 10,
        out_specs=hbm,
        scratch_shapes=[
            pltpu.VMEM((6, DM, 16, DH), BF16),
            pltpu.VMEM((3 * H * WP + 352, DH), U32),
            pltpu.VMEM((H * DH, DM), BF16),
            pltpu.VMEM((3, DF, S), BF16),
            pltpu.VMEM((352, 128), F32),
            pltpu.VMEM((6 * 16 * FP + 160, 128), F32),
            pltpu.VMEM((8, 64, 128), U32),
            pltpu.VMEM((8, 64, 128), U32),
            pltpu.VMEM((48, 64, 128), U32),
            pltpu.VMEM((48, 64, 128), U32),
            pltpu.VMEM((S, DM), F32),
            pltpu.VMEM((S, DM), BF16),
            pltpu.VMEM((S, DM), F32),
            pltpu.VMEM((16, 256, 384), F32),
            pltpu.VMEM((SEG, DM), F32),
            pltpu.VMEM((SEG, DM), F32),
            pltpu.VMEM((AHEAD + 32, DM), BF16),
            pltpu.VMEM((3, RING, H * DH), F32),
            pltpu.SemaphoreType.DMA((15,)),
        ],
        compiler_params=pltpu.CompilerParams(vmem_limit_bytes=120 * 1024 * 1024),
    )(A_x.reshape(S, DM), A_mem0.reshape(M, DM), A_Wq, A_Wk, A_Wv, A_Wo.reshape(H * DH, DM),
      B_w_r.T, B_w_i.T, *_dft_constants())
    return out.reshape(1, S, DM)
```

```python
import math

import jax
import jax.numpy as jnp
import ml_dtypes
import numpy as np
from jax.experimental import pallas as pl
from jax.experimental.pallas import tpu as pltpu

S, DM, H, DH, M, SEG = 2048, 640, 32, 128, 8, 32
L = M + SEG
NSEG = S // SEG
DF = DM // 2 + 1
G = 4
NG = H // G
AHEAD, RING = 288, 384
HEAD = 448
CU = 8
WP, FP = 321, 129
F32, BF16, U32 = jnp.float32, jnp.bfloat16, jnp.uint32
C1, C2 = math.cos(2 * math.pi / 5), math.cos(4 * math.pi / 5)
S1, S2 = math.sin(2 * math.pi / 5), math.sin(4 * math.pi / 5)


def _dft_constants():
    def mul3(f):
        return [f.real, f.real + f.imag, f.imag - f.real]

    def unit(n, period):
        return np.exp(2j * np.pi * (n % period) / period)

    def row_pairs(mats):
        a = np.stack(mats).reshape(-1, 64, 2, 128).astype(ml_dtypes.bfloat16).view(np.uint16).astype(np.uint32)
        return a[:, :, 0] | a[:, :, 1] << 16

    n2 = np.arange(128)
    scale = 2.0 / (DM * S)
    k = 5 * n2
    f = unit(n2[:, None] * k, DM) * (k <= DM // 2)
    edge = k % (DM // 2) == 0
    f = np.where(edge, f.real, f)
    w = np.where(edge, 0.5, 1.0)[:, None] * scale
    fwd, inv = [f.real, -f.imag], [w * f.T.real, -w * f.T.imag]
    for r in (1, 2):
        k = np.where(n2 < 64, r + 5 * n2, DM - (5 - r + 5 * (n2 - 64)))
        f = unit(n2[:, None] * k, DM)
        fwd += mul3(f)
        inv += mul3(scale * f.T)
    sf, si = [], []
    for k1 in range(16):
        f = unit((k1 + 16 * n2)[:, None] * n2, S)
        sf += mul3(f.conj())
        si += mul3(f.T)
    return row_pairs(fwd), row_pairs(inv), row_pairs(sf), row_pairs(si)


def _mm(a, b):
    return jnp.dot(a, b, preferred_element_type=F32)


def _layernorm(x):
    m = jnp.sum(x, axis=-1, keepdims=True) * (1.0 / DM)
    xc = x - m
    v = jnp.sum(xc * xc, axis=-1, keepdims=True) * (1.0 / DM)
    return xc * jax.lax.rsqrt(v + 1e-5)


def _tiles(x):
    return [x[:, i * 128:(i + 1) * 128] for i in range(x.shape[1] // 128)]


def _radix5(x):
    x0, x1, x2, x3, x4 = _tiles(x)
    a1, a2, b1, b2 = x1 + x4, x2 + x3, x1 - x4, x2 - x3
    return jnp.concatenate([x0 + a1 + a2,
                            x0 + C1 * a1 + C2 * a2, S1 * b1 + S2 * b2,
                            x0 + C2 * a1 + C1 * a2, S2 * b1 - S1 * b2], axis=1)


def _inv_radix5(t0, t1r, t1i, t2r, t2i):
    a1, b1 = t0 + C1 * t1r + C2 * t2r, S1 * t1i + S2 * t2i
    a2, b2 = t0 + C2 * t1r + C1 * t2r, S2 * t1i - S1 * t2i
    return jnp.concatenate([t0 + t1r + t2r, a1 - b1, a2 - b2, a2 + b2, a1 + b1], axis=1)


def _dft4(z, sign):
    (ar, ai), (br, bi), (cr, ci), (dr, di) = z
    pr, pi, mr, mi = ar + cr, ai + ci, ar - cr, ai - ci
    qr, qi, nr, ni = br + dr, bi + di, br - dr, bi - di
    lo, hi = (mr + ni, mi - nr), (mr - ni, mi + nr)
    if sign > 0:
        lo, hi = hi, lo
    return [(pr + qr, pi + qi), lo, (pr - qr, pi - qi), hi]


def _twiddle16(z, e, sign):
    zr, zi = z
    if e == 0:
        return z
    if e == 4:
        return (-zi, zr) if sign > 0 else (zi, -zr)
    c, s = math.cos(math.pi * e / 8), sign * math.sin(math.pi * e / 8)
    if e in (2, 6):
        if c * s > 0:
            return (zr - zi) * c, (zr + zi) * c
        return (zr + zi) * c, (zi - zr) * c
    return zr * c - zi * s, zr * s + zi * c


def _dft16(z, sign):
    u = [_dft4([z[4 * a + b] for a in range(4)], sign) for b in range(4)]
    out = [None] * 16
    for c in range(4):
        v = _dft4([_twiddle16(u[b][c], b * c, sign) for b in range(4)], sign)
        for d in range(4):
            out[c + 4 * d] = v[d]
    return out


def _kernel(x_hbm, mem_hbm, wq_hbm, wk_hbm, wv_hbm, wo_hbm, wr_hbm, wi_hbm,
            df_hbm, di_hbm, sf_hbm, si_hbm, out_hbm,
            raw_ref, w_ref, wo_ref, flt_raw, tmp_ref, flt_ref,
            df_ref, di_ref, sf_ref, si_ref,
            x_ref, io_ref, r_ref, u_ref, hn_ref, ao_ref, hb_ref, qkv_ref, sems):
    head, rest = pl.ds(0, HEAD), pl.ds(HEAD, S - HEAD)
    copies = [pltpu.make_async_copy(src, dst, sems.at[i]) for i, (src, dst) in enumerate(
        [(w.at[:, pl.ds(16 * j, 16), :], raw_ref.at[2 * i + j])
         for i, w in enumerate((wq_hbm, wk_hbm, wv_hbm)) for j in range(2)]
        + [(wo_hbm, wo_ref), (x_hbm.at[rest], io_ref.at[rest]),
           (wr_hbm, flt_raw.at[0]), (wi_hbm, flt_raw.at[1]),
           (df_hbm, df_ref), (di_hbm, di_ref), (sf_hbm, sf_ref), (si_hbm, si_ref),
           (x_hbm.at[head], io_ref.at[head]), (mem_hbm, hb_ref.at[pl.ds(AHEAD, M)])])]

    def rows(i, n):
        return pl.ds(pl.multiple_of(i * n, n), n)

    def weights(i, g, k):
        tiles = [w_ref[pl.ds((i * 32 + hd // 16 * 16 + hd % 2 * 8 + hd % 16 // 2) * WP + k * 64, 64), :]
                 for hd in range(g * G, (g + 1) * G)]
        return pltpu.bitcast(jnp.concatenate(tiles, axis=1), BF16)

    def project(h, i, g, between=None):
        acc = None
        for k in range(DM // 128):
            t = _mm(h[:, k * 128:(k + 1) * 128], weights(i, g, k))
            acc = t if acc is None else acc + t
            if between:
                between(g % 4 * 5 + k)
        return acc

    def load_rows(rs):
        x = io_ref[rs, :].astype(F32)
        x_ref[rs, :] = x
        return x

    def repack(i, j, c):
        v = pltpu.bitcast(raw_ref[2 * i + j, rows(c, 32)].reshape(32 * 16, DH), U32)
        for q in range(16):
            e, o = v[16 * q:16 * q + 8], v[16 * q + 8:16 * q + 16]
            at = (2 * i + j) * 16 * WP + c * 16 + q
            w_ref[pl.ds(at, 8, stride=WP), :] = (e & 0xFFFF) | (o << 16)
            w_ref[pl.ds(at + 8 * WP, 8, stride=WP), :] = (e >> 16) | (o & np.uint32(0xFFFF0000))

    copies[14].start()
    copies[0].start()
    flt_raw[2, :, :128] = jnp.zeros((DF, 128), BF16)
    ao_ref[...] = jnp.zeros((SEG, DM), F32)
    copies[14].wait()

    @pl.loop(0, AHEAD // 48)
    def _(c):
        hb_ref[rows(c, 48), :] = _layernorm(load_rows(rows(c, 48))).astype(BF16)

    load_rows(pl.ds(AHEAD, HEAD - AHEAD))
    copies[1].start()
    copies[15].start()
    copies[0].wait()
    pl.loop(0, DM // 32)(lambda c: repack(0, 0, c))

    @pl.loop(0, 3)
    def _(i):
        for j in range(2):
            def project_ahead(rs, between=None):
                for g in range(j * NG // 2, (j + 1) * NG // 2):
                    qkv_ref[i, rs, g * G * DH:(g + 1) * G * DH] = project(
                        hb_ref[rs, :], i, g, between)

            for n in range(j, 5, 2):
                pl.when(i == n // 2)(copies[n + 2].start)
            for c in range(AHEAD // 96 - 1):
                project_ahead(pl.ds(c * 96, 96))
            for n in range(j, 5, 2):
                pl.when(i == n // 2)(copies[n + 1].wait)
            project_ahead(pl.ds(AHEAD - 96, 96), lambda c: repack(jnp.minimum(i + j, 2), 1 - j, c))

    copies[6].wait()
    copies[15].wait()
    for c in copies[7:14]:
        c.start()

    def prepare_filter(p, c):
        blk = pl.ds(pl.multiple_of(c * 128, 128), 128)
        tmp_ref[:DF - 1, :] = flt_raw[p, :DF - 1, blk].astype(F32)
        last = jnp.concatenate([flt_raw[p, DF - 1:, blk].astype(F32), jnp.zeros((63, 128), F32)], axis=0)
        part = [tmp_ref[pl.ds(k, 64, stride=5), :] for k in range(5)]
        for r in range(3):
            v = jnp.concatenate([part[r], part[5 - r] if r else last], axis=0).T
            for q in range(16):
                at = ((p % 2 * 3 + r) * 16 + q % 2 * 8) * FP + c * 8 + q // 2
                flt_ref[pl.ds(at, 8, stride=FP), :] = v[8 * q:8 * q + 8]

    def enter(rs):
        hn_ref[...] = _layernorm(x_ref[rs, :])

    def leave(s):
        x = x_ref[rows(s, SEG), :] + ao_ref[...]
        x_ref[rows(s, SEG), :] = x
        r_ref[rows(s, SEG), :] = _radix5(_layernorm(x))

    ri = jax.lax.broadcasted_iota(jnp.int32, (L, L), 0)
    ci = jax.lax.broadcasted_iota(jnp.int32, (L, L), 1)
    mask = (ri < M) | (ri >= ci)

    def segment(s, mem, early):
        h = jnp.concatenate([mem, hn_ref[:SEG - M if early else SEG, :]], axis=0)
        leave(jnp.maximum(s - 1, 0))
        if early:
            enter(pl.ds(pl.multiple_of(AHEAD + (s + 1) * (SEG - M), 8), SEG))
            load_rows(rows(jnp.clip(HEAD // 64 + s - 4, HEAD // 64 - 1, S // 64 - 1), 64))
            piece = jnp.clip(s - 4, 0, 31)
            prepare_filter(jnp.where(s < 4, 2, piece // 16), piece % 16)
            put = pl.ds(pl.multiple_of((AHEAD + s * (SEG - M)) % RING, 8), SEG - M)
            get = pl.ds(pl.multiple_of(s * SEG % RING, SEG), SEG)
        else:
            enter(rows(jnp.minimum(s + 1, NSEG - 1), SEG))

        def proj(i, g):
            y = project(h.astype(BF16) if early else h, i, g)
            if early:
                cols = slice(g * G * DH, (g + 1) * G * DH)
                qkv_ref[i, put, cols] = y[M:]
                y = jnp.concatenate([y[:M], qkv_ref[i, get, cols]], axis=0)
            return y

        def scores(q, k):
            res = []
            for qh, kh in zip(_tiles(q), _tiles(k)):
                sc = jax.lax.dot_general(qh, kh.astype(BF16), (((1,), (1,)), ((), ())),
                                         preferred_element_type=F32)
                sc = jnp.where(mask, sc * DH ** -0.5, -1e9)
                e = jnp.exp(sc - jnp.max(sc, axis=-1, keepdims=True))
                d = jnp.sum(e, axis=-1, keepdims=True)
                r = pltpu.reciprocal(d, approx=True)
                res.append((e, r * (2.0 - d * r)))
            return res

        def values(es, v):
            return jnp.concatenate(
                [_mm(e, vh.astype(BF16)) * r for (e, r), vh in zip(es, _tiles(v))], axis=1)

        def project_out(out, g):
            t = _mm(os_[g], wo_ref[g * G * DH:(g + 1) * G * DH, :])
            return t if out is None else out + t

        lag = NG if early else 4
        os_, es, v, out = [], None, None, None
        for g in range(NG):
            q, k = proj(0, g), proj(1, g)
            if g:
                os_.append(values(es, v))
            v = proj(2, g)
            es = scores(q, k)
            if g >= lag:
                out = project_out(out, g - lag)
        for g in range(NG - lag, NG - 2):
            out = project_out(out, g)
        os_.append(values(es, v))
        for g in range(NG - 2, NG):
            out = project_out(out, g)
        ao_ref[...] = out[M:]
        return out[:M]

    def segments(first, last, mem, early):
        unroll = 2 if early else 4

        def body(i, mem):
            if early:
                @pl.when(i == 4 // unroll)
                def _():
                    for c in copies[7:10]:
                        c.wait()
            for q in range(unroll):
                mem = segment(i * unroll + q, mem, early)
            return mem
        return jax.lax.fori_loop(first // unroll, last // unroll, body, mem)

    def out_copy(c):
        rs = rows(c, 512)
        return pltpu.make_async_copy(io_ref.at[rs], out_hbm.at[rs], sems.at[c])

    def factor(ref, i):
        return pltpu.bitcast(ref[i], BF16)

    def times(zr, zi, ref, i):
        k = _mm(zr + zi, factor(ref, i))
        return k - _mm(zi, factor(ref, i + 1)), k + _mm(zr, factor(ref, i + 2))

    def applied(ref, i, zr, zi):
        k = _mm(factor(ref, i), (zr + zi).astype(BF16))
        return k - _mm(factor(ref, i + 1), zi.astype(BF16)), k + _mm(factor(ref, i + 2), zr.astype(BF16))

    def spectral(layer):
        sign = jnp.where(jax.lax.broadcasted_iota(jnp.int32, (1, 128), 1) < 64, 1.0, -1.0)

        @pl.loop(0, 16 // CU)
        def _(i):
            for q in range(CU):
                c = i * CU + q
                t0, t1r, t1i, t2r, t2i = _tiles(jnp.concatenate(
                    [r_ref[rows(n1 * 16 + c, 8), :] for n1 in range(16)], axis=0))
                y1, y2 = times(t1r, t1i, df_ref, 2), times(t2r, t2i, df_ref, 5)
                y0 = _mm(t0, factor(df_ref, 0)), _mm(t0, factor(df_ref, 1))
                for r, (yr, yi) in ((1, y1), (2, y2), (0, y0)):
                    yi = yi * -sign if r else yi
                    z = _dft16([(yr[n1 * 8:(n1 + 1) * 8], yi[n1 * 8:(n1 + 1) * 8]) for n1 in range(16)], -1)
                    for k1 in range(16):
                        for p in range(2):
                            u_ref[k1, rows(16 * p + c, 8), r * 128:(r + 1) * 128] = z[k1][p]

        @pl.loop(0, 2)
        def _(i):
            ys = []
            for q in range(8 + 2):
                if q < 8:
                    k1 = i * 8 + q
                    xr, xi = applied(sf_ref, 3 * k1, u_ref[k1, :128], u_ref[k1, 128:])
                    wr, wi = (jnp.concatenate([flt_ref[pl.ds(((p * 3 + r) * 16 + k1) * FP, 128), :]
                                               for r in range(3)], axis=1) for p in range(2))
                    ys.append((xr * wr - xi * wi, xr * wi + xi * wr))
                if q >= 2:
                    qkv_ref[i, :256, (q - 2) * 384:(q - 1) * 384] = jnp.concatenate(
                        applied(si_ref, 3 * (i * 8 + q - 2), *ys[q - 2]), axis=0)

        @pl.loop(0, 16)
        def _(c):
            for r in range(3):
                z = _dft16([[qkv_ref[k1 // 8, rows(16 * p + c, 8), pl.ds(k1 % 8 * 384 + r * 128, 128)]
                             for p in range(2)] for k1 in range(16)], 1)
                for n1 in range(16):
                    for p in range(2):
                        u_ref[n1, rows(16 * p + c, 8), r * 128:(r + 1) * 128] = z[n1][p]

        @pl.loop(0, 4)
        def _(i):
            for q in range(8):
                zr, zi = (_tiles(u_ref[i * 4 + q // 2, pl.ds(128 * p + q % 2 * 64, 64), :]) for p in range(2))
                t0 = _mm(zr[0], factor(di_ref, 0)) + _mm(zi[0], factor(di_ref, 1))
                rs = rows(i * 8 + q, 64)
                x = x_ref[rs, :] + _inv_radix5(t0, *times(zr[1], zi[1] * sign, di_ref, 2),
                                               *times(zr[2], zi[2] * sign, di_ref, 5))
                x_ref[rs, :] = x
                io_ref[rs, :] = x.astype(BF16)
            pl.when(layer == 1)(lambda: out_copy(i).start())

    mem0 = hb_ref[AHEAD:AHEAD + M, :].astype(F32)
    enter(pl.ds(AHEAD, SEG))
    mem1 = segments(0, AHEAD // M, mem0, True)
    for c in copies[10:14]:
        c.wait()

    @pl.loop(0, 2)
    def _(layer):
        first = jnp.where(layer == 0, AHEAD // M, 0)
        enter(rows(first, SEG))
        segments(first, NSEG, jnp.where(layer == 0, mem1, mem0), False)
        leave(NSEG - 1)
        ao_ref[...] = jnp.zeros((SEG, DM), F32)
        spectral(layer)

    for i in range(4):
        out_copy(i).wait()


@jax.jit
def pallas_interleave_layers__memory_aug_recurrent_mem_tr__spectral_gfnet__prompt_kernel(
    A_x: jax.Array,
    A_mem0: jax.Array,
    A_Wq: jax.Array,
    A_Wk: jax.Array,
    A_Wv: jax.Array,
    A_Wo: jax.Array,
    A_seg_len: jax.Array,
    B_x: jax.Array,
    B_w_r: jax.Array,
    B_w_i: jax.Array,
):
    del A_seg_len, B_x
    assert A_x.shape == (1, S, DM) and A_mem0.shape == (1, M, DM) and A_Wq.shape == (DM, H, DH)
    hbm = pl.BlockSpec(memory_space=pltpu.HBM)
    out = pl.pallas_call(
        _kernel,
        out_shape=jax.ShapeDtypeStruct((S, DM), BF16),
        in_specs=[hbm] * 12,
        out_specs=hbm,
        scratch_shapes=[
            pltpu.VMEM((6, DM, 16, DH), BF16),
            pltpu.VMEM((3 * H * WP + 352, DH), U32),
            pltpu.VMEM((H * DH, DM), BF16),
            pltpu.VMEM((3, DF, S), BF16),
            pltpu.VMEM((352, 128), F32),
            pltpu.VMEM((6 * 16 * FP + 160, 128), F32),
            pltpu.VMEM((8, 64, 128), U32),
            pltpu.VMEM((8, 64, 128), U32),
            pltpu.VMEM((48, 64, 128), U32),
            pltpu.VMEM((48, 64, 128), U32),
            pltpu.VMEM((S, DM), F32),
            pltpu.VMEM((S, DM), BF16),
            pltpu.VMEM((S, DM), F32),
            pltpu.VMEM((16, 256, 384), F32),
            pltpu.VMEM((SEG, DM), F32),
            pltpu.VMEM((SEG, DM), F32),
            pltpu.VMEM((AHEAD + 32, DM), BF16),
            pltpu.VMEM((3, RING, H * DH), F32),
            pltpu.SemaphoreType.DMA((16,)),
        ],
        compiler_params=pltpu.CompilerParams(vmem_limit_bytes=120 * 1024 * 1024),
    )(A_x.reshape(S, DM), A_mem0.reshape(M, DM), A_Wq, A_Wk, A_Wv, A_Wo.reshape(H * DH, DM),
      B_w_r.T, B_w_i.T, *_dft_constants())
    return out.reshape(1, S, DM)
```
